```python
import jax
import jax.numpy as jnp

def _softmax(x, axis=-1):
    return jax.nn.softmax(x, axis=axis)
def _gelu(x):
    return jax.nn.gelu(x, approximate=True)
def _silu(x):
    return jax.nn.silu(x)
def _sigmoid(x):
    return jax.nn.sigmoid(x)
def _layernorm(x, axis=-1, eps=1e-5):
    m = jnp.mean(x, axis=axis, keepdims=True)
    v = jnp.var(x, axis=axis, keepdims=True)
    return (x - m) / jnp.sqrt(v + eps)
def _scatter_add(tgt, idx, src, axis=0):
    return tgt.at[idx].add(src)
def _segment_sum(src, seg, n):
    return jax.ops.segment_sum(src, seg, n)
class _Rng:
    def __init__(self, key):
        self._k = key
    def _next(self):
        self._k, sub = jax.random.split(self._k)
        return sub
    def normal(self, shape):
        return jax.random.normal(self._next(), shape, dtype=jnp.bfloat16)
    def randint(self, lo, hi, shape):
        return jax.random.randint(self._next(), shape, lo, hi, dtype=jnp.int32)
    def uniform(self, shape, lo=0.0, hi=1.0):
        return jax.random.uniform(self._next(), shape, jnp.bfloat16, lo, hi)
    def permutation(self, n):
        return jax.random.permutation(self._next(), n)


kernel_name = 'standalone__modern_conv_block_slak__vision'

def setup_inputs():
    _rng = _Rng(jax.random.key(int.from_bytes(__import__("os").urandom(4), "little")))
    _w = (lambda a: (lambda t: t.astype(jnp.bfloat16) if jnp.issubdtype(t.dtype, jnp.floating) else t)(jnp.asarray(a)))
    H = W = 384
    C = 384
    K = 1
    return {
        "x": _w((lambda *s: _rng.normal(s) * 0.05)(1, H, W, C)),
        "dw": _w((lambda *s: _rng.normal(s) * 0.05)(K, K, C)),
        "w1": _w((lambda *s: _rng.normal(s) * 0.05)(C, 4 * C)),
        "w2": _w((lambda *s: _rng.normal(s) * 0.05)(4 * C, C)),
        "grn_g": _w((lambda *s: _rng.normal(s) * 0.05)(4 * C)),
        "grn_b": _w((lambda *s: _rng.normal(s) * 0.05)(4 * C)),
    }

def reference(x, dw, w1, w2, grn_g, grn_b):
    B, H, W, C = x.shape
    K = dw.shape[0]
    pad = K // 2
    xp = jnp.pad(x, ((0,0),(pad,pad),(pad,pad),(0,0)))
    out = jnp.zeros_like(x)
    for i in range(K):
        for j in range(K):
            out = out + xp[:, i:i+H, j:j+W, :] * dw[i, j][None, None, None, :]
    h = _layernorm(out, axis=-1)
    h = _gelu(h @ w1)
    gx = jnp.sqrt((h * h).sum(axis=(1, 2), keepdims=True) + 1e-6)
    nx = gx / (gx.mean(axis=-1, keepdims=True) + 1e-6)
    h = grn_g[None, None, None, :] * (h * nx) + grn_b[None, None, None, :] + h
    return x + h @ w2
```

```python
import functools, math
import numpy as np
import jax, jax.numpy as jnp
from jax import lax
from jax.experimental import pallas as pl
from jax.experimental.pallas import tpu as pltpu

F32, BF16 = jnp.float32, jnp.bfloat16
_C0 = math.sqrt(2.0 / math.pi)
_C1 = 0.044715 * _C0

def build(TM=1024, R=30, NB=3, NX=3, CM1=256, CN1=1536, CM2=256, vmem=126, phase=3, nodma=0):
    def fn(x, dw, w1, w2, grn_g, grn_b):
        B, H, W, C = x.shape
        N = B * H * W
        F = w1.shape[1]
        T = N // TM
        K = T - R
        def kernel(x_hbm, dw_ref, w1_ref, w2_ref, g_ref, b_ref, o_hbm, h_hbm,
                   xbuf, obuf, hv, w1s, w2s, xsem, osem, hsem):
            def xcp(t, s): return pltpu.make_async_copy(x_hbm.at[pl.ds(pl.multiple_of(t * TM, TM), TM)], xbuf.at[s], xsem.at[s])
            def ocp(t, s): return pltpu.make_async_copy(obuf.at[s], o_hbm.at[pl.ds(pl.multiple_of(t * TM, TM), TM)], osem.at[s])
            def hw(k, s): return pltpu.make_async_copy(hv.at[R + s], h_hbm.at[k], hsem.at[s])
            def hr(k, s): return pltpu.make_async_copy(h_hbm.at[k], hv.at[R + s], hsem.at[s])
            def place(t):
                r = (t * R) // T
                res = ((t + 1) * R) // T != r
                k = t - r
                ring = k % NB
                return res, k, ring, jnp.where(res, r, R + ring)

            for i in range(NX - 1):
                xcp(i, i).start()
            w1s[...] = (w1_ref[...].astype(F32) * 0.5).astype(BF16)
            dwv = dw_ref[...].astype(F32)

            def p1(t, acc):
                res, k, ring, slot = place(t)
                xs = t % NX
                @pl.when(t + NX - 1 < T)
                def _():
                    xcp(t + NX - 1, (t + NX - 1) % NX).start()
                xcp(t, xs).wait()
                if not nodma:
                    @pl.when(jnp.logical_and(jnp.logical_not(res), k >= NB))
                    def _():
                        hw(k - NB, ring).wait()
                accs = list(acc)
                for c in range(TM // CM1):
                    rows = pl.ds(c * CM1, CM1)
                    o = xbuf[xs, rows, :].astype(F32) * dwv
                    m = jnp.mean(o, axis=-1, keepdims=True)
                    d = o - m
                    v = jnp.mean(d * d, axis=-1, keepdims=True)
                    xn = (d * lax.rsqrt(v + 1e-5)).astype(BF16)
                    for j in range(F // CN1):
                        cols = pl.ds(j * CN1, CN1)
                        z = jnp.dot(xn, w1s[:, cols], preferred_element_type=F32)
                        u = z * (z * z * (8.0 * _C1) + (2.0 * _C0))
                        hh = z + z * jnp.tanh(u)
                        hv[slot, rows, cols] = hh.astype(BF16)
                        accs[j] = accs[j] + jnp.sum((hh * hh).reshape(CM1 // 8, 8, CN1), axis=0)
                if not nodma:
                    @pl.when(jnp.logical_and(jnp.logical_not(res), k < K - NB))
                    def _():
                        hw(k, ring).start()
                return tuple(accs)

            acc0 = tuple(jnp.zeros((8, CN1), F32) for _ in range(F // CN1))
            if phase & 1:
                acc = lax.fori_loop(0, T, p1, acc0)
            else:
                acc = acc0
                for i in range(NX - 1):
                    xcp(i, i).wait()
            if not (phase & 2):
                obuf[0, 0:8, :] = sum(a[:, 0:C] for a in acc).astype(BF16)
                ocp(0, 0).start(); ocp(0, 0).wait()
                return
            for i in range(NX - 1):
                xcp(T - 1 - i, i).start()
            ss = jnp.sum(jnp.concatenate(acc, axis=1), axis=0, keepdims=True)
            gx = jnp.sqrt(ss + 1e-6)
            nx = gx / (jnp.mean(gx, axis=-1, keepdims=True) + 1e-6)
            s = 1.0 + g_ref[...].astype(F32) * nx
            st = jnp.transpose(jnp.broadcast_to(s, (128, F)))
            for j in range(C // 128):
                w2s[:, j * 128:(j + 1) * 128] = (w2_ref[:, j * 128:(j + 1) * 128].astype(F32) * st).astype(BF16)
            bias = jnp.dot(jnp.broadcast_to(b_ref[...], (16, F)), w2_ref[...], preferred_element_type=F32)[0:1]

            def p2(i, carry):
                t = T - 1 - i
                res, k, ring, slot = place(t)
                xs = i % NX
                os_ = i % 2
                @pl.when(i + NX - 1 < T)
                def _():
                    xcp(t - (NX - 1), (i + NX - 1) % NX).start()
                xcp(t, xs).wait()
                if not nodma:
                    @pl.when(jnp.logical_and(jnp.logical_not(res), k < K - NB))
                    def _():
                        hr(k, ring).wait()
                @pl.when(i >= 2)
                def _():
                    ocp(t + 2, os_).wait()
                for c in range(TM // CM2):
                    rows = pl.ds(c * CM2, CM2)
                    y = jnp.dot(hv[slot, rows, :], w2s[...], preferred_element_type=F32)
                    obuf[os_, rows, :] = (xbuf[xs, rows, :].astype(F32) + bias + y).astype(BF16)
                ocp(t, os_).start()
                if not nodma:
                    @pl.when(jnp.logical_and(jnp.logical_not(res), k >= NB))
                    def _():
                        hr(k - NB, ring).start()
                return carry
            lax.fori_loop(0, T, p2, 0)
            ocp(1, T % 2).wait()
            ocp(0, (T - 1) % 2).wait()

        vm = pl.BlockSpec(memory_space=pltpu.VMEM)
        hb = pl.BlockSpec(memory_space=pl.ANY)
        out, _ = pl.pallas_call(
            kernel,
            in_specs=[hb, vm, vm, vm, vm, vm],
            out_specs=[hb, hb],
            out_shape=[jax.ShapeDtypeStruct((N, C), x.dtype), jax.ShapeDtypeStruct((K - NB, TM, F), BF16)],
            scratch_shapes=[
                pltpu.VMEM((NX, TM, C), BF16), pltpu.VMEM((2, TM, C), BF16),
                pltpu.VMEM((R + NB, TM, F), BF16),
                pltpu.VMEM((C, F), BF16), pltpu.VMEM((F, C), BF16),
                pltpu.SemaphoreType.DMA((NX,)), pltpu.SemaphoreType.DMA((2,)), pltpu.SemaphoreType.DMA((NB,)),
            ],
            compiler_params=pltpu.CompilerParams(vmem_limit_bytes=vmem * 1024 * 1024),
        )(x.reshape(N, C), dw.reshape(1, C), w1, w2, grn_g.reshape(1, F), grn_b.reshape(1, F))
        return out.reshape(x.shape)
    return fn


@jax.jit
def pallas_standalone__modern_conv_block_slak__vision_kernel(x, dw, w1, w2, grn_g, grn_b):
    return build()(x, dw, w1, w2, grn_g, grn_b)
```

```python
import math
import jax, jax.numpy as jnp
from jax import lax
from jax.experimental import pallas as pl
from jax.experimental.pallas import tpu as pltpu

F32, BF16, U32 = jnp.float32, jnp.bfloat16, jnp.uint32
_C0 = math.sqrt(2.0 / math.pi)
_C1 = 0.044715 * _C0
_AL = _C1 ** (1.0 / 3.0)
_CC = _C0 / _AL
_HS = 0.5 / _AL
L = 128

_BF = [
    [(1, 0, 0), (1, 0, 2), (1, 1, 0)], [(1, 0, 0), (-1, 0, 1), (1, 2, 0)], [(-1, 1, 0), (1, 1, 1), (1, 2, 1)],
    [(-1, 0, 1), (-1, 1, 1), (-1, 1, 2)], [(1, 1, 2), (1, 2, 0), (1, 2, 2)], [(1, 0, 2), (1, 2, 1), (1, 2, 2)],
    [(1, 0, 1), (1, 1, 0)], [(-1, 1, 0)], [(1, 0, 1)],
    [(-1, 0, 2), (1, 2, 0)], [(1, 0, 2)], [(-1, 2, 0)],
    [(1, 1, 2), (-1, 2, 1)], [(-1, 1, 2)], [(-1, 2, 1)],
]

def lincomb(terms, blk):
    acc = None
    for sg, k, n in sorted(terms, reverse=True):
        v = blk(k, n)
        acc = (v if sg > 0 else -v) if acc is None else (acc + v if sg > 0 else acc - v)
    return acc

def a_forms(x, y):
    x1, x2, x3 = x; y1, y2, y3 = y
    s1 = x1 + y1; s2 = x2 + y2
    f13 = s1 - y3; f23 = s2 - x3
    return {1: x1, 2: s1, 3: s2, 4: y2, 5: x3, 6: y3, 7: x1 + y2, 8: x1 - x2, 9: y1 - y2,
            10: f13, 11: y1 - y3, 12: f13 - x3, 13: f23, 14: x2 - x3, 15: f23 - y3}

def pk(v): return v.astype(BF16)
def upk(v): return pltpu.bitcast(v, BF16)
def f32(v): return v.astype(F32)

def hk1(M, out):
    m10 = M(10); m11 = M(11); m1 = M(1); m12 = M(12)
    g13 = m10 + m11; d1 = m1 + g13; t1 = d1 + m12; t2 = g13 + m12
    m5 = M(5); m14 = M(14); m8 = M(8); m13 = M(13)
    out(m5 - t2 - m14, 0, 2); out(t1 + m8, 0, 0)
    g23 = m13 + m14; v3 = m11 + g23
    m6 = M(6); m15 = M(15); m9 = M(9); m4 = M(4)
    d2 = g23 + m4
    out(v3 + m6 - m15, 1, 2); out(m9 + m15 - d2, 1, 1)
    v1 = m9 - d1; u2 = d2 + m8
    m2 = M(2); m3 = M(3); m7 = M(7)
    out(v1 + m2 + m7, 1, 0); out(u2 + m3 + m7, 0, 1)

def hk2(MM, M9, out):
    def chain(a, b, c):
        def f(ld):
            e = f32(ld(*b)) - f32(ld(*c))
            return pk(f32(ld(*a)) + e), pk(e)
        return f
    def sums(k):
        def f(ld):
            s = f32(ld(0, k)) + f32(ld(1, k))
            return pk(s), pk(s - (f32(ld(0, 2)) + f32(ld(1, 2))))
        return f
    def f78(ld):
        x1 = f32(ld(0, 0))
        return pk(x1 + f32(ld(1, 1))), pk(x1 - f32(ld(0, 1)))
    m1, m5 = MM(1, 5, lambda ld: (ld(0, 0), ld(0, 2)))
    m10, m11 = MM(10, 11, chain((0, 0), (1, 0), (1, 2)))
    g13 = m10 + m11; d1 = m1 + g13; u3 = m5 - g13
    m2, m12 = MM(2, 12, sums(0))
    v1 = m2 - d1; u1 = d1 + m12; u3 = u3 - m12
    m4, m6 = MM(4, 6, lambda ld: (ld(1, 1), ld(1, 2)))
    v3 = m6 + m11
    m13, m14 = MM(13, 14, chain((1, 1), (0, 1), (0, 2)))
    g23 = m13 + m14; d2 = m4 + g23; v3 = v3 + g23
    out(u3 - m14, 0, 2)
    m3, m15 = MM(3, 15, sums(1))
    u2 = d2 + m3; v2 = m15 - d2
    out(v3 - m15, 1, 2)
    m7, m8 = MM(7, 8, f78)
    out(u1 + m8, 0, 0); out(u2 + m7 + m8, 0, 1)
    v1 = v1 + m7
    m9 = M9(lambda ld: pk(f32(ld(1, 0)) - f32(ld(1, 1))))
    out(v1 + m9, 1, 0); out(v2 + m9, 1, 1)

def build(TM=1024, S=40, NB=4, PR=32, CM2=256, vmem=128, phase=3, nodma=0, head=0, newfirst=1, sep=1, xp=0, op=0, NX=3, hp=1, wp=0):
    def fn(x, dw, w1, w2, grn_g, grn_b):
        B, H, W, C = x.shape
        N = B * H * W
        F = w1.shape[1]
        T = N // TM
        R = S - NB
        K = T - R
        NT = F // L
        NP = TM // (2 * PR)
        NC2 = TM // (2 * CM2)
        def kernel(x_hbm, dw_ref, w1_hbm, w2_hbm, g_ref, b_ref, o_hbm, h_hbm,
                   xbuf, hv, wf, af, xsem, osem, hsem, wsem):
            def xcp(t): return pltpu.make_async_copy(x_hbm.at[pl.ds(pl.multiple_of(t * TM, TM), TM)], xbuf.at[t % NX], xsem.at[t % NX])
            def ocp(t): return pltpu.make_async_copy(xbuf.at[t % NX], o_hbm.at[pl.ds(pl.multiple_of(t * TM, TM), TM)], osem.at[t % NX])
            def hw(k): return pltpu.make_async_copy(hv.at[R + k % NB], h_hbm.at[k], hsem.at[k % NB])
            def hr(k): return pltpu.make_async_copy(h_hbm.at[k], hv.at[R + k % NB], hsem.at[k % NB])
            def place(t):
                r = (t * R) // T
                stream = ((t + 1) * R) // T == r
                k = t - r
                return stream, k, jnp.where(stream, R + k % NB, r)
            wf32, af32, hv32 = wf.bitcast(U32), af.bitcast(U32), hv.bitcast(U32)
            def wtile(r, g): return upk(wf32[r - 1, g * 64:(g + 1) * 64, :])

            w1cp = [pltpu.make_async_copy(w1_hbm.at[:, pl.ds(j * L, L)], hv.at[R - 1, j, pl.ds(0, C)], wsem.at[0]) for j in range(NT)]
            xcp(0).start()
            for cp in w1cp: cp.start()
            xcp(1).start()
            af[...] = jnp.zeros(af.shape, BF16)
            dwv = f32(dw_ref[...])

            def piece(xs, q, ring):
                o = f32(xbuf[xs, pl.ds(2 * PR * q, 2 * PR), :]) * dwv
                d = o - jnp.sum(o, axis=-1, keepdims=True) * (1.0 / C)
                v = jnp.sum(d * d, axis=-1, keepdims=True)
                xn = d * (lax.rsqrt(v + C * 1e-5) * (_AL * math.sqrt(C)))
                A = a_forms([xn[:PR, i * L:(i + 1) * L] for i in range(3)], [xn[PR:, i * L:(i + 1) * L] for i in range(3)])
                for r in range(1, 16):
                    af[ring, r - 1] = pk(A[r])

            def unit(u, qs, slot, prev, accs):
                g = u % 4
                def M(r):
                    a = jnp.concatenate([af32[q % 8, r - 1] for q in qs], axis=0)
                    return jnp.dot(upk(a), wtile(r, g), preferred_element_type=F32)
                def out(y, half, n):
                    j = 4 * n + g
                    hh = y + y * jnp.tanh(y * (y * y + _CC))
                    hb = pk(hh)
                    for i, q in enumerate(qs):
                        hv[slot if q >= 0 else prev, j, pl.ds(((q % NP) * 2 + half) * PR, PR), :] = hb[i * PR:(i + 1) * PR]
                    accs[j] = accs[j] + jnp.sum((hh * hh).reshape(-1, 8, L), axis=0)
                hk1(M, out)

            xcp(0).wait()
            if not head: piece(0, 0, 0)
            for cp in w1cp: cp.wait()
            for r, terms in enumerate(_BF):
                for g in range(4):
                    wf[r, g * L:(g + 1) * L, :] = pk(lincomb(terms, lambda k, n: f32(hv[R - 1, 4 * n + g, k * L:(k + 1) * L, :])))

            def p1(t, acc):
                stream, k, slot = place(t)
                pstream, pk_, prev = place(jnp.maximum(t - 1, 0))
                if not nodma & 2:
                    @pl.when(t + 2 < T)
                    def _():
                        xcp(t + 2).start()
                    @pl.when(t + 1 < T)
                    def _():
                        xcp(t + 1).wait()
                if not nodma & 1:
                    @pl.when(jnp.logical_and(stream, k >= NB))
                    def _():
                        hw(k - NB).wait()
                accs = list(acc)
                for u in range(NP):
                    if head: piece(t % NX, u, u % 8)
                    elif u + 1 < NP: piece(t % NX, u + 1, (u + 1) % 8)
                    else: piece(jnp.minimum(t + 1, T - 1) % NX, 0, 0)
                    qs = [u, u - 1, u - 2, u - 3]
                    if not newfirst or (head and u == 0): qs = qs[::-1]
                    unit(u, qs, slot, prev, accs)
                if not nodma & 1:
                    @pl.when(jnp.logical_and(jnp.logical_and(pstream, t > 0), pk_ < K - NB))
                    def _():
                        hw(pk_).start(priority=wp)
                return tuple(accs)

            acc = tuple(jnp.zeros((8, L), F32) for _ in range(NT))
            if phase & 1:
                accs = list(lax.fori_loop(0, T, p1, acc))
                last = place(T - 1)[2]
                for u in range(3):
                    unit(u, [q for q in range(u - 3, 0)], last, last, accs)
                acc = accs
            else:
                xcp(1).wait()
            if nodma & 2 and phase & 1: xcp(1).wait()
            if not (phase & 2):
                xbuf[0, 0:8, 0:L] = sum(acc).astype(BF16)
                ocp(0).start(); ocp(0).wait()
                return
            w2cp = [pltpu.make_async_copy(w2_hbm.at[pl.ds(i * F // 2, F // 2)], xbuf.at[(T + i) % NX, pl.ds(0, F // 2)], wsem.at[i]) for i in range(2)]
            for cp in w2cp: cp.start()
            ss = jnp.sum(jnp.concatenate(acc, axis=1), axis=0, keepdims=True) * (_HS * _HS)
            gx = jnp.sqrt(ss + 1e-6)
            nx = gx / (jnp.mean(gx, axis=-1, keepdims=True) + 1e-6)
            s = (1.0 + f32(g_ref[...]) * nx) * _HS
            st = jnp.transpose(jnp.broadcast_to(s, (L, F)))
            for cp in w2cp: cp.wait()
            def w2rows(r0, n, cols):
                return xbuf[(T + r0 // (F // 2)) % NX, pl.ds(r0 % (F // 2), n), cols]
            for r, terms in enumerate(_BF):
                for g in range(4):
                    blk = lambda k, n: f32(w2rows((4 * k + g) * L, L, slice(n * L, (n + 1) * L))) * st[(4 * k + g) * L:(4 * k + g + 1) * L]
                    wf[r, g * L:(g + 1) * L, :] = pk(lincomb(terms, blk))
            bb = jnp.broadcast_to(b_ref[...], (16, F))
            bias = sum(jnp.dot(bb[:, i * F // 2:(i + 1) * F // 2], w2rows(i * F // 2, F // 2, slice(None)), preferred_element_type=F32) for i in range(2))[0:1]

            def p2(i, carry):
                t = T - 1 - i
                stream, k, slot = place(t)
                xs = t % NX
                if not nodma & 2:
                    @pl.when(i >= 2)
                    def _():
                        ocp(t + 2).wait()
                    @pl.when(t >= NX - 2)
                    def _():
                        xcp(t - (NX - 2)).start(priority=xp)
                    @pl.when(i >= NX - 2)
                    def _():
                        xcp(t).wait()
                if not nodma & 1:
                    @pl.when(jnp.logical_and(stream, k < K - NB))
                    def _():
                        hr(k).wait()
                for c in range(NC2):
                    def loader(z, g):
                        sl = slot + (i // (T + z) if sep else 0)
                        return lambda half, kk: upk(hv32[sl, 4 * kk + g, pl.ds((2 * c + half) * (CM2 // 2), CM2 // 2), :])
                    dt = lambda a, r, g: jnp.dot(a, wtile(r, g), preferred_element_type=F32)
                    def MM(ra, rb, f):
                        ya = yb = None
                        for g in (0, 2):
                            o = [f(loader(ra, gg)) for gg in (g, g + 1)]
                            a = dt(o[0][0], ra, g) + dt(o[1][0], ra, g + 1)
                            b = dt(o[0][1], rb, g) + dt(o[1][1], rb, g + 1)
                            ya, yb = (a, b) if ya is None else (ya + a, yb + b)
                        return ya, yb
                    def M9(f):
                        d = [dt(f(loader(9, g)), 9, g) for g in range(4)]
                        return (d[0] + d[1]) + (d[2] + d[3])
                    def out(y, half, n):
                        rows = pl.ds((2 * c + half) * CM2, CM2); cols = slice(n * L, (n + 1) * L)
                        xbuf[xs, rows, cols] = (f32(xbuf[xs, rows, cols]) + bias[:, cols] + y).astype(BF16)
                    hk2(MM, M9, out)
                if not nodma & 2: ocp(t).start(priority=op)
                if not nodma & 1:
                    @pl.when(jnp.logical_and(stream, k >= NB))
                    def _():
                        hr(k - NB).start(priority=hp)
                return carry
            lax.fori_loop(0, T, p2, 0)
            if not nodma & 2: ocp(1).wait()
            else: ocp(0).start()
            ocp(0).wait()

        vm = pl.BlockSpec(memory_space=pltpu.VMEM)
        hb = pl.BlockSpec(memory_space=pl.ANY)
        out, _ = pl.pallas_call(
            kernel,
            in_specs=[hb, vm, hb, hb, vm, vm],
            out_specs=[hb, hb],
            out_shape=[jax.ShapeDtypeStruct((N, C), x.dtype), jax.ShapeDtypeStruct((K - NB, NT, TM, L), BF16)],
            scratch_shapes=[
                pltpu.VMEM((NX, TM, C), BF16),
                pltpu.VMEM((S, NT, TM, L), BF16),
                pltpu.VMEM((15, 512, L), BF16),
                pltpu.VMEM((8, 15, PR, L), BF16),
                pltpu.SemaphoreType.DMA((NX,)), pltpu.SemaphoreType.DMA((NX,)), pltpu.SemaphoreType.DMA((NB,)),
                pltpu.SemaphoreType.DMA((2,)),
            ],
            compiler_params=pltpu.CompilerParams(vmem_limit_bytes=vmem * 1024 * 1024),
        )(x.reshape(N, C), dw.reshape(1, C), w1, w2, grn_g.reshape(1, F), grn_b.reshape(1, F))
        return out.reshape(x.shape)
    return fn


@jax.jit
def pallas_standalone__modern_conv_block_slak__vision_kernel(x, dw, w1, w2, grn_g, grn_b):
    return build()(x, dw, w1, w2, grn_g, grn_b)
```

```python
import math
import jax, jax.numpy as jnp
from jax import lax
from jax.experimental import pallas as pl
from jax.experimental.pallas import tpu as pltpu

F32, BF16, U32 = jnp.float32, jnp.bfloat16, jnp.uint32
_C0 = math.sqrt(2.0 / math.pi)
_C1 = 0.044715 * _C0
_AL = _C1 ** (1.0 / 3.0)
_CC = _C0 / _AL
_HS = 0.5 / _AL
L = 128

_BF = [
    [(1, 0, 0), (1, 0, 2), (1, 1, 0)], [(1, 0, 0), (-1, 0, 1), (1, 2, 0)], [(-1, 1, 0), (1, 1, 1), (1, 2, 1)],
    [(-1, 0, 1), (-1, 1, 1), (-1, 1, 2)], [(1, 1, 2), (1, 2, 0), (1, 2, 2)], [(1, 0, 2), (1, 2, 1), (1, 2, 2)],
    [(1, 0, 1), (1, 1, 0)], [(-1, 1, 0)], [(1, 0, 1)],
    [(-1, 0, 2), (1, 2, 0)], [(1, 0, 2)], [(-1, 2, 0)],
    [(1, 1, 2), (-1, 2, 1)], [(-1, 1, 2)], [(-1, 2, 1)],
]

def lincomb(terms, blk):
    acc = None
    for sg, k, n in sorted(terms, reverse=True):
        v = blk(k, n)
        acc = (v if sg > 0 else -v) if acc is None else (acc + v if sg > 0 else acc - v)
    return acc

def a_forms(x, y):
    x1, x2, x3 = x; y1, y2, y3 = y
    s1 = x1 + y1; s2 = x2 + y2
    f13 = s1 - y3; f23 = s2 - x3
    return {1: x1, 2: s1, 3: s2, 4: y2, 5: x3, 6: y3, 7: x1 + y2, 8: x1 - x2, 9: y1 - y2,
            10: f13, 11: y1 - y3, 12: f13 - x3, 13: f23, 14: x2 - x3, 15: f23 - y3}

def pk(v): return v.astype(BF16)
def upk(v): return pltpu.bitcast(v, BF16)
def f32(v): return v.astype(F32)

def hk1(M, out, mid, perm):
    m = {}
    def issue(*rs):
        k = len(m)
        for i in sorted(range(len(rs)), key=lambda i: perm[k + i]): m[rs[i]] = M(rs[i])
    def outs(k, a, b):
        for o in ((a, b) if perm[15 + k] < 0.5 else (b, a)): out(*o)
    issue(10, 11, 1, 12); mid(0)
    g13 = m[10] + m[11]; d1 = m[1] + g13; t1 = d1 + m[12]; t2 = g13 + m[12]
    issue(5, 14, 8, 13); mid(1)
    outs(0, (m[5] - t2 - m[14], 0, 2), (t1 + m[8], 0, 0))
    g23 = m[13] + m[14]; v3 = m[11] + g23
    issue(6, 15, 9, 4); mid(2)
    d2 = g23 + m[4]
    outs(1, (v3 + m[6] - m[15], 1, 2), (m[9] + m[15] - d2, 1, 1))
    v1 = m[9] - d1; u2 = d2 + m[8]
    issue(2, 3, 7); mid(3)
    outs(2, (v1 + m[2] + m[7], 1, 0), (u2 + m[3] + m[7], 0, 1))
    mid(4)

def hk2(MM, M9, out):
    def chain(a, b, c):
        def f(ld):
            e = f32(ld(*b)) - f32(ld(*c))
            return pk(f32(ld(*a)) + e), pk(e)
        return f
    def sums(k):
        def f(ld):
            s = f32(ld(0, k)) + f32(ld(1, k))
            return pk(s), pk(s - (f32(ld(0, 2)) + f32(ld(1, 2))))
        return f
    def f78(ld):
        x1 = f32(ld(0, 0))
        return pk(x1 + f32(ld(1, 1))), pk(x1 - f32(ld(0, 1)))
    m1, m5 = MM(1, 5, lambda ld: (ld(0, 0), ld(0, 2)))
    m10, m11 = MM(10, 11, chain((0, 0), (1, 0), (1, 2)))
    g13 = m10 + m11; d1 = m1 + g13; u3 = m5 - g13
    m2, m12 = MM(2, 12, sums(0))
    v1 = m2 - d1; u1 = d1 + m12; u3 = u3 - m12
    m4, m6 = MM(4, 6, lambda ld: (ld(1, 1), ld(1, 2)))
    v3 = m6 + m11
    m13, m14 = MM(13, 14, chain((1, 1), (0, 1), (0, 2)))
    g23 = m13 + m14; d2 = m4 + g23; v3 = v3 + g23
    out(u3 - m14, 0, 2)
    m3, m15 = MM(3, 15, sums(1))
    u2 = d2 + m3; v2 = m15 - d2
    out(v3 - m15, 1, 2)
    m7, m8 = MM(7, 8, f78)
    out(u1 + m8, 0, 0); out(u2 + m7 + m8, 0, 1)
    v1 = v1 + m7
    m9 = M9(lambda ld: pk(f32(ld(1, 0)) - f32(ld(1, 1))))
    out(v1 + m9, 1, 0); out(v2 + m9, 1, 1)

def build(S=40, PR=32, CM2=256, vmem=128, phase=3, nodma=0, hp=1, sep=1, nocomp=0, Q=10, XD=2, AR=4, pf=4, seed=1, rs=1, fl=0, ord1=0, qo=0, sg=0, un2=1, nb=1, wp=0, NE=2, pair=0):
    TM, U1 = 1024, 2
    import random
    rnd = random.Random(seed)
    perm = [rnd.random() for _ in range(18)] if seed else list(range(15)) + [0, 0, 0]
    qord = [0, 1, 2, 3]
    if seed and qo: rnd.shuffle(qord)
    def fn(x, dw, w1, w2, grn_g, grn_b):
        B, H, W, C = x.shape
        N = B * H * W
        F = w1.shape[1]
        T = N // TM
        NT = F // L
        PS = 2 * PR
        NP = TM // PS
        J = T // U1
        NC2 = TM // (2 * CM2)
        def kernel(x_hbm, dw_ref, w1_hbm, w2_hbm, g_ref, b_ref, o_hbm, h_hbm,
                   hv, wf, w2v, xbuf, xp, af, xsem, osem, hsem, psem, wsem, esem):
            def rows(ref, t): return ref.at[pl.ds(pl.multiple_of(t * TM, TM), TM)]
            def xcp(t): return pltpu.make_async_copy(rows(x_hbm, t), xbuf.at[t & 3], xsem.at[t & 3])
            def ocp(t): return pltpu.make_async_copy(xbuf.at[t & 3], rows(o_hbm, t), osem.at[t & 3])
            def pcp(j): return pltpu.make_async_copy(x_hbm.at[pl.ds(pl.multiple_of(j * U1 * TM, TM), PS)], xp.at[j & 1], psem.at[j & 1])
            def hw(t, sl): return pltpu.make_async_copy(hv.at[sl], h_hbm.at[t], hsem.at[sl])
            def hr(t, sl): return pltpu.make_async_copy(h_hbm.at[t], hv.at[sl], hsem.at[sl])
            def nxt(sl): return jnp.where(sl == S - 1, 0, sl + 1)
            def prv(sl): return jnp.where(sl == 0, S - 1, sl - 1)
            wf32, hv32, af32 = wf.bitcast(U32), hv.bitcast(U32), af.bitcast(U32)
            def wtile(r, g): return upk(wf32[r - 1, g * 64:(g + 1) * 64, :])

            w1cp = [pltpu.make_async_copy(w1_hbm.at[:, pl.ds(j * L, L)], hv.at[S - 1, j, pl.ds(0, C)], wsem.at[j % 4]) for j in range(NT)]
            w2cp = pltpu.make_async_copy(w2_hbm, w2v, wsem.at[4])
            pcp(0).start()
            for g in range(4):
                for n in range(3): w1cp[4 * n + g].start()
            xcp(0).start(); xcp(1).start(); pcp(1).start(); xcp(2).start(); xcp(3).start()
            w2cp.start()
            af[...] = jnp.zeros(af.shape, BF16)
            dwv = f32(dw_ref[...])

            def piece(xv, ring):
                o = f32(xv) * dwv
                d = o - jnp.sum(o, axis=-1, keepdims=True) * (1.0 / C)
                v = jnp.sum(d * d, axis=-1, keepdims=True)
                if rs == 0: rstd = lax.rsqrt(v + C * 1e-5) * (_AL * math.sqrt(C))
                if rs == 1: rstd = jnp.exp2(jnp.log2(v + C * 1e-5) * -0.5 + math.log2(_AL * math.sqrt(C)))
                if rs == 2: rstd = jnp.exp(jnp.log(v + C * 1e-5) * -0.5 + math.log(_AL * math.sqrt(C)))
                xn = d * rstd
                A = a_forms([xn[:PR, i * L:(i + 1) * L] for i in range(3)], [xn[PR:, i * L:(i + 1) * L] for i in range(3)])
                for r in range(1, 16):
                    af[ring, r - 1] = pk(A[r])

            def unit(u, qs, slots, accs, mid=lambda k: None):
                g = u % 4
                def M(r):
                    a = jnp.concatenate([af32[q % AR, r - 1] for q in qs], axis=0)
                    return jnp.dot(upk(a), wtile(r, g), preferred_element_type=F32)
                def out(y, half, n):
                    j = 4 * n + g
                    hh = y * lax.logistic(y * (y * y + _CC)) if sg else y + y * jnp.tanh(y * (y * y + _CC))
                    hb = pk(hh)
                    for i, q in enumerate(qs):
                        hv[slots[q // NP], j, pl.ds(((q % NP) * 2 + half) * PR, PR), :] = hb[i * PR:(i + 1) * PR]
                    accs[j] = accs[j] + jnp.sum((hh * hh).reshape(-1, 8, L), axis=0)
                hk1(M, out, mid, perm)

            pcp(0).wait()
            piece(xp[0], 0)
            pcp(2).start()
            for g in range(4):
                for n in range(3): w1cp[4 * n + g].wait()
                blk = {(k, n): f32(hv[S - 1, 4 * n + g, k * L:(k + 1) * L, :]) for k in range(3) for n in range(3)}
                for r, terms in enumerate(_BF):
                    wf[r, g * L:(g + 1) * L, :] = pk(lincomb(terms, lambda k, n: blk[k, n]))

            def step1(j, carry):
                s0, acc = carry
                t0 = j * U1
                slots = {-1: prv(s0), 0: s0, 1: nxt(s0)}
                accs = list(acc)
                for u in range(U1 * NP):
                    def mid(k):
                        if k != pf: return
                        q = u + 1
                        if q < U1 * NP: piece(xbuf[(t0 + q // NP) & 3, pl.ds((q % NP) * PS, PS), :], q % AR)
                        else: piece(xp[(j + 1) & 1], 0)
                    unit(u, [u - d for d in qord], slots, accs, mid)
                for e in (-1, 0):
                    @pl.when(jnp.logical_and(t0 + e >= 0, t0 + e < T - S))
                    def _():
                        hw(t0 + e, slots[e]).start(priority=wp)
                @pl.when(j + 2 < J)
                def _():
                    for e in range(U1): xcp(t0 + 2 * U1 + e).start()
                @pl.when(j + 3 < J)
                def _():
                    pcp(j + 3).start()
                @pl.when(j + 1 < J)
                def _():
                    for e in range(U1): xcp(t0 + U1 + e).wait()
                @pl.when(j + 2 < J)
                def _():
                    pcp(j + 2).wait()
                s2 = nxt(slots[1])
                @pl.when(jnp.logical_and(t0 + U1 >= S, j + 1 < J))
                def _():
                    hw(t0 + U1 - S, s2).wait()
                    hw(t0 + U1 + 1 - S, nxt(s2)).wait()
                return s2, tuple(accs)

            acc = tuple(jnp.zeros((8, L), F32) for _ in range(NT))
            xcp(0).wait(); xcp(1).wait(); pcp(1).wait()
            if phase & 1:
                accs = list(lax.fori_loop(0, J, step1, (jnp.int32(0), acc))[1])
                for u in range(3):
                    unit(u, list(range(u - 3, 0)), {-1: (T - 1) % S}, accs)
                acc = accs
            else:
                xcp(2).wait(); xcp(3).wait(); pcp(2).wait()
            w2cp.wait()
            if not phase & 2:
                xbuf[0, 0:8, 0:L] = sum(acc).astype(BF16)
                ocp(0).start(); ocp(0).wait()
                return

            ss = jnp.sum(jnp.concatenate(acc, axis=1), axis=0, keepdims=True)
            gx = jnp.sqrt(ss * (_HS * _HS) + 1e-6)
            nx = gx / (jnp.mean(gx, axis=-1, keepdims=True) + 1e-6)
            s = (1.0 + f32(g_ref[...]) * nx) * _HS
            for g in range(4):
                blk = {}
                for k in range(3):
                    j = 4 * k + g
                    st = jnp.transpose(jnp.broadcast_to(s[:, j * L:(j + 1) * L], (L, L)))
                    for n in range(3):
                        blk[k, n] = f32(w2v[j * L:(j + 1) * L, n * L:(n + 1) * L]) * st
                for r, terms in enumerate(_BF):
                    wf[r, g * L:(g + 1) * L, :] = pk(lincomb(terms, lambda k, n: blk[k, n]))
            bias = jnp.dot(jnp.broadcast_to(b_ref[...], (16, F)), w2v[...], preferred_element_type=F32)[0:1]

            def chunk(i, slot, xs, r0, cm):
                def loader(z, g):
                    sl = slot + (i >> (8 + z))
                    return lambda half, kk: upk(hv32[sl, 4 * kk + g, pl.ds(pl.multiple_of((r0 + half * cm) // 2, cm // 2), cm // 2), :])
                dt = lambda a, r, g: jnp.dot(a, wtile(r, g), preferred_element_type=F32)
                def MM(ra, rb, f):
                    ya = yb = None
                    for g in (0, 2):
                        o = [f(loader(ra, gg)) for gg in (g, g + 1)]
                        a = dt(o[0][0], ra, g) + dt(o[1][0], ra, g + 1)
                        b = dt(o[0][1], rb, g) + dt(o[1][1], rb, g + 1)
                        ya, yb = (a, b) if ya is None else (ya + a, yb + b)
                    return ya, yb
                def M9(f):
                    d = [dt(f(loader(9, g)), 9, g) for g in range(4)]
                    return (d[0] + d[1]) + (d[2] + d[3])
                def out(y, half, n):
                    rr = pl.ds(pl.multiple_of(r0 + half * cm, cm), cm); cols = slice(n * L, (n + 1) * L)
                    xbuf[xs, rr, cols] = (f32(xbuf[xs, rr, cols]) + bias[:, cols] + y).astype(BF16)
                hk2(MM, M9, out)

            PE = TM // NE
            def hpart(t, sl, c, sem):
                part = pl.ds(pl.multiple_of(c * PE, PE), PE)
                return pltpu.make_async_copy(h_hbm.at[t, :, part], hv.at[sl, :, part], sem)

            def first(c, _):
                chunk(c, (T - 1) % S, (T - 1) & 3, c * PE, PE // 2)
                hpart(T - S - 1, (T - 1) % S, c, hsem.at[(T - 1) % S]).start(priority=hp)
            lax.fori_loop(0, NE, first, None)
            if not pair: ocp(T - 1).start()

            def step2(i, carry, second):
                slot, m, ms, err = carry
                t = T - 1 - i
                for c in range(0 if nocomp else NC2):
                    chunk(i, slot, t & 3, 2 * c * CM2, CM2)
                if not pair: ocp(t).start()
                elif second: ocp(t + 1).start(); ocp(t).start()
                err = err + (T - S)
                go = jnp.logical_and(err >= T - Q, m >= 0)
                @pl.when(jnp.logical_and(go, m > 0))
                def _():
                    hr(m, ms).start(priority=hp)
                @pl.when(jnp.logical_and(go, m == 0))
                def _():
                    for c in range(NE): hpart(0, 0, c, esem.at[c]).start(priority=hp)
                if not pair:
                    ocp(t + 1).wait()
                    @pl.when(t >= 3)
                    def _():
                        xcp(t - 3).start()
                    @pl.when(i >= 3)
                    def _():
                        xcp(t - 1).wait()
                elif second:
                    @pl.when(i >= 3)
                    def _():
                        xcp(t - 1).wait(); xcp(t - 2).wait()
                else:
                    ocp(t + 2).wait(); ocp(t + 1).wait()
                    @pl.when(t >= 3)
                    def _():
                        xcp(t - 2).start(); xcp(t - 3).start()
                @pl.when(jnp.logical_and(i >= S - 1, t >= 2))
                def _():
                    hr(t - 1, prv(slot)).wait()
                return prv(slot), jnp.where(go, m - 1, m), jnp.where(go, prv(ms), ms), jnp.where(go, err - (T - Q), err)
            i32 = jnp.int32
            def steps2(j, c):
                for e in range(un2): c = step2(1 + j * un2 + e, c, e == 0)
                return c
            lax.fori_loop(0, (T - 2) // un2, steps2, (i32((T - 2) % S), i32(T - S - 2), i32((T - 2) % S), i32(T - Q - 1)))

            if pair: ocp(1).start()
            def last(c, _):
                hpart(0, 0, c, esem.at[c]).wait()
                chunk(c, 0, 0, c * PE, PE // 2)
                part = pl.ds(pl.multiple_of(c * PE, PE), PE)
                pltpu.make_async_copy(xbuf.at[0, part], o_hbm.at[part], osem.at[0]).start()
            lax.fori_loop(0, NE, last, None)
            ocp(1).wait(); ocp(0).wait()

        vm = pl.BlockSpec(memory_space=pltpu.VMEM)
        hb = pl.BlockSpec(memory_space=pl.ANY)
        out, _ = pl.pallas_call(
            kernel,
            in_specs=[hb, vm, hb, hb, vm, vm],
            out_specs=[hb, hb],
            out_shape=[jax.ShapeDtypeStruct((N, C), x.dtype), jax.ShapeDtypeStruct((T - S, NT, TM, L), BF16)],
            scratch_shapes=[
                pltpu.VMEM((S, NT, TM, L), BF16),
                pltpu.VMEM((15, 512, L), BF16),
                pltpu.VMEM((F, C), BF16),
                pltpu.VMEM((4, TM, C), BF16),
                pltpu.VMEM((2, PS, C), BF16),
                pltpu.VMEM((AR, 15, PR, L), BF16),
                pltpu.SemaphoreType.DMA((4,)), pltpu.SemaphoreType.DMA((4,)), pltpu.SemaphoreType.DMA((S,)),
                pltpu.SemaphoreType.DMA((2,)), pltpu.SemaphoreType.DMA((5,)), pltpu.SemaphoreType.DMA((NE,)),
            ],
            compiler_params=pltpu.CompilerParams(vmem_limit_bytes=vmem * 1024 * 1024, disable_bounds_checks=bool(nb), flags={n: True for i, n in enumerate(["XLA_TPU_FORCE_LP_LLO_SCHEDULER", "XLA_TPU_EVENLY_DISTRIBUTE_CRITICAL_NODES", "XLA_TPU_RESCHEDULE_DMA_DONES"]) if fl >> i & 1} or None),
        )(x.reshape(N, C), dw.reshape(1, C), w1, w2, grn_g.reshape(1, F), grn_b.reshape(1, F))
        return out.reshape(x.shape)
    return fn


@jax.jit
def pallas_standalone__modern_conv_block_slak__vision_kernel(x, dw, w1, w2, grn_g, grn_b):
    return build()(x, dw, w1, w2, grn_g, grn_b)
```

```python
import math
import jax, jax.numpy as jnp
from jax import lax
from jax.experimental import pallas as pl
from jax.experimental.pallas import tpu as pltpu

F32, BF16, U32 = jnp.float32, jnp.bfloat16, jnp.uint32
_C0 = math.sqrt(2.0 / math.pi)
_C1 = 0.044715 * _C0
_AL = _C1 ** (1.0 / 3.0)
_CC = _C0 / _AL
_HS = 0.5 / _AL
L = 128

_BF = [
    [(1, 0, 0), (1, 0, 2), (1, 1, 0)], [(1, 0, 0), (-1, 0, 1), (1, 2, 0)], [(-1, 1, 0), (1, 1, 1), (1, 2, 1)],
    [(-1, 0, 1), (-1, 1, 1), (-1, 1, 2)], [(1, 1, 2), (1, 2, 0), (1, 2, 2)], [(1, 0, 2), (1, 2, 1), (1, 2, 2)],
    [(1, 0, 1), (1, 1, 0)], [(-1, 1, 0)], [(1, 0, 1)],
    [(-1, 0, 2), (1, 2, 0)], [(1, 0, 2)], [(-1, 2, 0)],
    [(1, 1, 2), (-1, 2, 1)], [(-1, 1, 2)], [(-1, 2, 1)],
]

def lincomb(terms, blk):
    acc = None
    for sg, k, n in sorted(terms, reverse=True):
        v = blk(k, n)
        acc = (v if sg > 0 else -v) if acc is None else (acc + v if sg > 0 else acc - v)
    return acc

def a_forms(x, y):
    x1, x2, x3 = x; y1, y2, y3 = y
    s1 = x1 + y1; s2 = x2 + y2
    f13 = s1 - y3; f23 = s2 - x3
    return {1: x1, 2: s1, 3: s2, 4: y2, 5: x3, 6: y3, 7: x1 + y2, 8: x1 - x2, 9: y1 - y2,
            10: f13, 11: y1 - y3, 12: f13 - x3, 13: f23, 14: x2 - x3, 15: f23 - y3}

def pk(v): return v.astype(BF16)
def upk(v): return pltpu.bitcast(v, BF16)
def f32(v): return v.astype(F32)

def hk1(M, out, mid, perm):
    m = {}
    def issue(*rs):
        k = len(m)
        for i in sorted(range(len(rs)), key=lambda i: perm[k + i]): m[rs[i]] = M(rs[i])
    def outs(k, a, b):
        for o in ((a, b) if perm[15 + k] < 0.5 else (b, a)): out(*o)
    issue(10, 11, 1, 12); mid(0)
    g13 = m[10] + m[11]; d1 = m[1] + g13; t1 = d1 + m[12]; t2 = g13 + m[12]
    issue(5, 14, 8, 13); mid(1)
    outs(0, (m[5] - t2 - m[14], 0, 2), (t1 + m[8], 0, 0))
    g23 = m[13] + m[14]; v3 = m[11] + g23
    issue(6, 15, 9, 4); mid(2)
    d2 = g23 + m[4]
    outs(1, (v3 + m[6] - m[15], 1, 2), (m[9] + m[15] - d2, 1, 1))
    v1 = m[9] - d1; u2 = d2 + m[8]
    issue(2, 3, 7); mid(3)
    outs(2, (v1 + m[2] + m[7], 1, 0), (u2 + m[3] + m[7], 0, 1))
    mid(4)

def hk2(MM, M9, out):
    def chain(a, b, c):
        def f(ld):
            e = f32(ld(*b)) - f32(ld(*c))
            return pk(f32(ld(*a)) + e), pk(e)
        return f
    def sums(k):
        def f(ld):
            s = f32(ld(0, k)) + f32(ld(1, k))
            return pk(s), pk(s - (f32(ld(0, 2)) + f32(ld(1, 2))))
        return f
    def f78(ld):
        x1 = f32(ld(0, 0))
        return pk(x1 + f32(ld(1, 1))), pk(x1 - f32(ld(0, 1)))
    m1, m5 = MM(1, 5, lambda ld: (ld(0, 0), ld(0, 2)))
    m10, m11 = MM(10, 11, chain((0, 0), (1, 0), (1, 2)))
    g13 = m10 + m11; d1 = m1 + g13; u3 = m5 - g13
    m2, m12 = MM(2, 12, sums(0))
    v1 = m2 - d1; u1 = d1 + m12; u3 = u3 - m12
    m4, m6 = MM(4, 6, lambda ld: (ld(1, 1), ld(1, 2)))
    v3 = m6 + m11
    m13, m14 = MM(13, 14, chain((1, 1), (0, 1), (0, 2)))
    g23 = m13 + m14; d2 = m4 + g23; v3 = v3 + g23
    out(u3 - m14, 0, 2)
    m3, m15 = MM(3, 15, sums(1))
    u2 = d2 + m3; v2 = m15 - d2
    out(v3 - m15, 1, 2)
    m7, m8 = MM(7, 8, f78)
    out(u1 + m8, 0, 0); out(u2 + m7 + m8, 0, 1)
    v1 = v1 + m7
    m9 = M9(lambda ld: pk(f32(ld(1, 0)) - f32(ld(1, 1))))
    out(v1 + m9, 1, 0); out(v2 + m9, 1, 1)

def build(S=40, PR=32, CM2=256, vmem=128, phase=3, nodma=0, hp=1, sep=1, nocomp=0, Q=10, XD=2, AR=4, pf=4, seed=1, rs=1, fl=0, ord1=0, qo=0, sg=0, un2=2, nb=1, wp=0, NE=2, pair=1, d1=1, man=1, P='302110231032201zzz_0321102310322010zz_032110231032201z00_012310231032201zzz', bk1=32, bk2=0):
    TM, U1 = 1024, 2
    import random
    rnd = random.Random(seed)
    perm = [rnd.random() for _ in range(18)] if seed else list(range(15)) + [0, 0, 0]
    qord = [0, 1, 2, 3]
    perms = [perm] * 4
    if P: perms = [[int(ch, 36) / 36 for ch in p] for p in P.split("_")]
    if seed and qo: rnd.shuffle(qord)
    def fn(x, dw, w1, w2, grn_g, grn_b):
        B, H, W, C = x.shape
        N = B * H * W
        F = w1.shape[1]
        T = N // TM
        NT = F // L
        PS = 2 * PR
        NP = TM // PS
        J = T // U1
        NC2 = TM // (2 * CM2)
        def kernel(x_hbm, dw_in, w1_hbm, w2_hbm, g_in, b_in, o_hbm, h_hbm,
                   hv, wf, w2v, xbuf, xp, af, xsem, osem, hsem, psem, wsem, esem, dw_v, g_v, b_v, ssem):
            dw_ref, g_ref, b_ref = (dw_v, g_v, b_v) if man else (dw_in, g_in, b_in)
            small = [pltpu.make_async_copy(a, b, ssem.at[i]) for i, (a, b) in enumerate(((dw_in, dw_v), (g_in, g_v), (b_in, b_v)))]
            def rows(ref, t): return ref.at[pl.ds(pl.multiple_of(t * TM, TM), TM)]
            def xcp(t): return pltpu.make_async_copy(rows(x_hbm, t), xbuf.at[t & 3], xsem.at[t & 3])
            def ocp(t): return pltpu.make_async_copy(xbuf.at[t & 3], rows(o_hbm, t), osem.at[t & 3])
            def pcp(j): return pltpu.make_async_copy(x_hbm.at[pl.ds(pl.multiple_of(j * U1 * TM, TM), PS)], xp.at[j & 1], psem.at[j & 1])
            def hw(t, sl): return pltpu.make_async_copy(hv.at[sl], h_hbm.at[t], hsem.at[sl])
            def hr(t, sl): return pltpu.make_async_copy(h_hbm.at[t], hv.at[sl], hsem.at[sl])
            def nxt(sl): return jnp.where(sl == S - 1, 0, sl + 1)
            def prv(sl): return jnp.where(sl == 0, S - 1, sl - 1)
            wf32, hv32, af32 = wf.bitcast(U32), hv.bitcast(U32), af.bitcast(U32)
            def wtile(r, g): return upk(wf32[r - 1, g * 64:(g + 1) * 64, :])

            w1cp = [pltpu.make_async_copy(w1_hbm.at[:, pl.ds(j * L, L)], hv.at[S - 1, j, pl.ds(0, C)], wsem.at[j % 4]) for j in range(NT)]
            w2cp = pltpu.make_async_copy(w2_hbm, w2v, wsem.at[4])
            pcp(0).start()
            if man: small[0].start()
            for g in range(4):
                for n in range(3): w1cp[4 * n + g].start()
            xcp(0).start(); xcp(1).start(); pcp(1).start(); xcp(2).start(); xcp(3).start()
            w2cp.start()
            if man: small[1].start(); small[2].start()
            af[...] = jnp.zeros(af.shape, BF16)
            if man: small[0].wait()
            dwv = f32(dw_ref[...])

            def piece(xv, ring):
                o = f32(xv) * dwv
                d = o - jnp.sum(o, axis=-1, keepdims=True) * (1.0 / C)
                v = jnp.sum(d * d, axis=-1, keepdims=True)
                if rs == 0: rstd = lax.rsqrt(v + C * 1e-5) * (_AL * math.sqrt(C))
                if rs == 1: rstd = jnp.exp2(jnp.log2(v + C * 1e-5) * -0.5 + math.log2(_AL * math.sqrt(C)))
                if rs == 2: rstd = jnp.exp(jnp.log(v + C * 1e-5) * -0.5 + math.log(_AL * math.sqrt(C)))
                xn = d * rstd
                A = a_forms([xn[:PR, i * L:(i + 1) * L] for i in range(3)], [xn[PR:, i * L:(i + 1) * L] for i in range(3)])
                for r in range(1, 16):
                    af[ring, r - 1] = pk(A[r])

            def unit(u, qs, slots, accs, mid=lambda k: None):
                g = u % 4
                def M(r):
                    a = jnp.concatenate([af32[q % AR, r - 1] for q in qs], axis=0)
                    return jnp.dot(upk(a), wtile(r, g), preferred_element_type=F32)
                def out(y, half, n):
                    j = 4 * n + g
                    hh = y * lax.logistic(y * (y * y + _CC)) if sg else y + y * jnp.tanh(y * (y * y + _CC))
                    hb = pk(hh)
                    for i, q in enumerate(qs):
                        hv[slots[q // NP], j, pl.ds(((q % NP) * 2 + half) * PR, PR), :] = hb[i * PR:(i + 1) * PR]
                    accs[j] = accs[j] + jnp.sum((hh * hh).reshape(-1, 8, L), axis=0)
                hk1(M, out, mid, perms[u % 4])

            pcp(0).wait()
            piece(xp[0], 0)
            pcp(2).start()
            for g in range(4):
                for n in range(3): w1cp[4 * n + g].wait()
                blk = {(k, n): f32(hv[S - 1, 4 * n + g, k * L:(k + 1) * L, :]) for k in range(3) for n in range(3)}
                for r, terms in enumerate(_BF):
                    wf[r, g * L:(g + 1) * L, :] = pk(lincomb(terms, lambda k, n: blk[k, n]))

            def step1(j, carry):
                s0, acc = carry
                t0 = j * U1
                slots = {-1: prv(s0), 0: s0, 1: nxt(s0)}
                accs = list(acc)
                s2 = nxt(slots[1])
                def book():
                    for e in (-1, 0):
                        @pl.when(jnp.logical_and(t0 + e >= 0, t0 + e < T - S))
                        def _():
                            hw(t0 + e, slots[e]).start(priority=wp)
                    @pl.when(j + 2 < J)
                    def _():
                        for e in range(U1): xcp(t0 + 2 * U1 + e).start()
                    @pl.when(j + 3 < J)
                    def _():
                        pcp(j + 3).start()
                def book2():
                    @pl.when(j + 1 < J)
                    def _():
                        for e in range(U1): xcp(t0 + U1 + e).wait()
                    @pl.when(j + 2 < J)
                    def _():
                        pcp(j + 2).wait()
                    @pl.when(jnp.logical_and(t0 + U1 >= S, j + 1 < J))
                    def _():
                        hw(t0 + U1 - S, s2).wait()
                        hw(t0 + U1 + 1 - S, nxt(s2)).wait()
                for u in range(U1 * NP):
                    if u == bk1: book()
                    def mid(k):
                        if k != pf: return
                        q = u + 1
                        if q < U1 * NP: piece(xbuf[(t0 + q // NP) & 3, pl.ds((q % NP) * PS, PS), :], q % AR)
                        else: piece(xp[(j + 1) & 1], 0)
                    unit(u, [u - d for d in qord], slots, accs, mid)
                if bk1 >= U1 * NP: book()
                book2()
                return s2, tuple(accs)

            acc = tuple(jnp.zeros((8, L), F32) for _ in range(NT))
            xcp(0).wait(); xcp(1).wait(); pcp(1).wait()
            if phase & 1:
                accs = list(lax.fori_loop(0, J, step1, (jnp.int32(0), acc))[1])
                for u in range(3):
                    unit(u, list(range(u - 3, 0)), {-1: (T - 1) % S}, accs)
                acc = accs
            else:
                xcp(2).wait(); xcp(3).wait(); pcp(2).wait()
            w2cp.wait()
            if man: small[1].wait(); small[2].wait()
            if not phase & 2:
                xbuf[0, 0:8, 0:L] = sum(acc).astype(BF16)
                ocp(0).start(); ocp(0).wait()
                return

            ss = jnp.sum(jnp.concatenate(acc, axis=1), axis=0, keepdims=True)
            gx = jnp.sqrt(ss * (_HS * _HS) + 1e-6)
            nx = gx / (jnp.mean(gx, axis=-1, keepdims=True) + 1e-6)
            s = (1.0 + f32(g_ref[...]).reshape(1, F) * nx) * _HS
            for g in range(4):
                blk = {}
                for k in range(3):
                    j = 4 * k + g
                    st = jnp.transpose(jnp.broadcast_to(s[:, j * L:(j + 1) * L], (L, L)))
                    for n in range(3):
                        blk[k, n] = f32(w2v[j * L:(j + 1) * L, n * L:(n + 1) * L]) * st
                for r, terms in enumerate(_BF):
                    wf[r, g * L:(g + 1) * L, :] = pk(lincomb(terms, lambda k, n: blk[k, n]))
            bias = jnp.dot(jnp.broadcast_to(f32(b_ref[...]).reshape(1, F), (16, F)).astype(BF16), w2v[...], preferred_element_type=F32)[0:1]

            def chunk(i, slot, xs, r0, cm):
                def loader(z, g):
                    sl = slot + (i >> (8 + z))
                    return lambda half, kk: upk(hv32[sl, 4 * kk + g, pl.ds(pl.multiple_of((r0 + half * cm) // 2, cm // 2), cm // 2), :])
                dt = lambda a, r, g: jnp.dot(a, wtile(r, g), preferred_element_type=F32)
                def MM(ra, rb, f):
                    ya = yb = None
                    for g in (0, 2):
                        o = [f(loader(ra, gg)) for gg in (g, g + 1)]
                        a = dt(o[0][0], ra, g) + dt(o[1][0], ra, g + 1)
                        b = dt(o[0][1], rb, g) + dt(o[1][1], rb, g + 1)
                        ya, yb = (a, b) if ya is None else (ya + a, yb + b)
                    return ya, yb
                def M9(f):
                    d = [dt(f(loader(9, g)), 9, g) for g in range(4)]
                    return (d[0] + d[1]) + (d[2] + d[3])
                def out(y, half, n):
                    rr = pl.ds(pl.multiple_of(r0 + half * cm, cm), cm); cols = slice(n * L, (n + 1) * L)
                    xbuf[xs, rr, cols] = (f32(xbuf[xs, rr, cols]) + bias[:, cols] + y).astype(BF16)
                hk2(MM, M9, out)

            PE = TM // NE
            def hpart(t, sl, c, sem):
                part = pl.ds(pl.multiple_of(c * PE, PE), PE)
                return pltpu.make_async_copy(h_hbm.at[t, :, part], hv.at[sl, :, part], sem)

            def first(c, _):
                chunk(c, (T - 1) % S, (T - 1) & 3, c * PE, PE // 2)
                hpart(T - S - 1, (T - 1) % S, c, hsem.at[(T - 1) % S]).start(priority=hp)
            lax.fori_loop(0, NE, first, None)
            if not pair: ocp(T - 1).start()

            def step2(i, carry, second):
                slot, m, ms, err = carry
                t = T - 1 - i
                for c in range(0 if nocomp else NC2):
                    chunk(i, slot, t & 3, 2 * c * CM2, CM2)
                if not pair: ocp(t).start()
                elif second: ocp(t + 1).start(); ocp(t).start()
                err = err + (T - S)
                go = jnp.logical_and(err >= T - Q, m >= 0)
                @pl.when(jnp.logical_and(go, m > 0))
                def _():
                    hr(m, ms).start(priority=hp)
                @pl.when(jnp.logical_and(go, m == 0))
                def _():
                    for c in range(NE): hpart(0, 0, c, esem.at[c]).start(priority=hp)
                if not pair:
                    ocp(t + 1).wait()
                    @pl.when(t >= 3)
                    def _():
                        xcp(t - 3).start()
                    @pl.when(i >= 3)
                    def _():
                        xcp(t - 1).wait()
                elif second:
                    @pl.when(i >= 3)
                    def _():
                        xcp(t - 1).wait(); xcp(t - 2).wait()
                else:
                    ocp(t + 2).wait(); ocp(t + 1).wait()
                    @pl.when(t >= 3)
                    def _():
                        xcp(t - 2).start(); xcp(t - 3).start()
                @pl.when(jnp.logical_and(i >= S - 1, t >= 2))
                def _():
                    hr(t - 1, prv(slot)).wait()
                return prv(slot), jnp.where(go, m - 1, m), jnp.where(go, prv(ms), ms), jnp.where(go, err - (T - Q), err)
            i32 = jnp.int32
            def steps2(j, c):
                for e in range(un2): c = step2(1 + j * un2 + e, c, e == 0)
                return c
            lax.fori_loop(0, (T - 2) // un2, steps2, (i32((T - 2) % S), i32(T - S - 2), i32((T - 2) % S), i32(T - Q - 1)))

            if pair: ocp(1).start()
            def last(c, _):
                hpart(0, 0, c, esem.at[c]).wait()
                chunk(c, 0, 0, c * PE, PE // 2)
                part = pl.ds(pl.multiple_of(c * PE, PE), PE)
                pltpu.make_async_copy(xbuf.at[0, part], o_hbm.at[part], osem.at[0]).start()
            lax.fori_loop(0, NE, last, None)
            ocp(1).wait(); ocp(0).wait()

        vm = pl.BlockSpec(memory_space=pltpu.VMEM)
        hb = pl.BlockSpec(memory_space=pl.ANY)
        out, _ = pl.pallas_call(
            kernel,
            in_specs=[hb] * 6 if man else [hb, vm, hb, hb, vm, vm],
            out_specs=[hb, hb],
            out_shape=[jax.ShapeDtypeStruct((N, C), x.dtype), jax.ShapeDtypeStruct((T - S, NT, TM, L), BF16)],
            scratch_shapes=[
                pltpu.VMEM((S, NT, TM, L), BF16),
                pltpu.VMEM((15, 512, L), BF16),
                pltpu.VMEM((F, C), BF16),
                pltpu.VMEM((4, TM, C), BF16),
                pltpu.VMEM((2, PS, C), BF16),
                pltpu.VMEM((AR, 15, PR, L), BF16),
                pltpu.SemaphoreType.DMA((4,)), pltpu.SemaphoreType.DMA((4,)), pltpu.SemaphoreType.DMA((S,)),
                pltpu.SemaphoreType.DMA((2,)), pltpu.SemaphoreType.DMA((5,)), pltpu.SemaphoreType.DMA((NE,)),
                pltpu.VMEM((1, C), dw.dtype), pltpu.VMEM((F,), grn_g.dtype), pltpu.VMEM((F,), grn_b.dtype), pltpu.SemaphoreType.DMA((3,)),
            ],
            compiler_params=pltpu.CompilerParams(vmem_limit_bytes=vmem * 1024 * 1024, disable_bounds_checks=bool(nb), flags={n: True for i, n in enumerate(["XLA_TPU_FORCE_LP_LLO_SCHEDULER", "XLA_TPU_EVENLY_DISTRIBUTE_CRITICAL_NODES", "XLA_TPU_RESCHEDULE_DMA_DONES"]) if fl >> i & 1} or None),
        )(x.reshape(N, C), dw.reshape(1, C), w1, w2, *((grn_g, grn_b) if d1 else (grn_g.reshape(1, F), grn_b.reshape(1, F))))
        return out.reshape(x.shape)
    return fn


@jax.jit
def pallas_standalone__modern_conv_block_slak__vision_kernel(x, dw, w1, w2, grn_g, grn_b):
    return build()(x, dw, w1, w2, grn_g, grn_b)
```

```python
import math

import jax
import jax.numpy as jnp
from jax import lax
from jax.experimental import pallas as pl
from jax.experimental.pallas import tpu as pltpu

F32, BF16, U32 = jnp.float32, jnp.bfloat16, jnp.uint32
L = 128
TM = 1024
S = 40
U1 = 2
PR = 32
CM = 256
NE = 2
LEAD = 10

_C0 = math.sqrt(2.0 / math.pi)
_AL = (0.044715 * _C0) ** (1.0 / 3.0)
_CC = _C0 / _AL
_HS = 0.5 / _AL

_B_FORMS = (
    ((1, 0, 0), (1, 0, 2), (1, 1, 0)),
    ((1, 0, 0), (-1, 0, 1), (1, 2, 0)),
    ((-1, 1, 0), (1, 1, 1), (1, 2, 1)),
    ((-1, 0, 1), (-1, 1, 1), (-1, 1, 2)),
    ((1, 1, 2), (1, 2, 0), (1, 2, 2)),
    ((1, 0, 2), (1, 2, 1), (1, 2, 2)),
    ((1, 0, 1), (1, 1, 0)),
    ((-1, 1, 0),),
    ((1, 0, 1),),
    ((-1, 0, 2), (1, 2, 0)),
    ((1, 0, 2),),
    ((-1, 2, 0),),
    ((1, 1, 2), (-1, 2, 1)),
    ((-1, 1, 2),),
    ((-1, 2, 1),),
)

_ORDER = (
    (((11, 12, 1, 10), (14, 5, 8, 13), (15, 6, 4, 9), (3, 7, 2)), (1, 1, 1)),
    (((10, 12, 1, 11), (14, 5, 8, 13), (15, 6, 4, 9), (3, 7, 2)), (0, 1, 1)),
    (((10, 12, 1, 11), (14, 5, 8, 13), (15, 6, 4, 9), (3, 7, 2)), (1, 0, 0)),
    (((10, 11, 1, 12), (14, 5, 8, 13), (15, 6, 4, 9), (3, 7, 2)), (1, 1, 1)),
)


def _bf16(v):
    return v.astype(BF16)


def _f32(v):
    return v.astype(F32)


def _words(v):
    return pltpu.bitcast(v, BF16)


def _b_form(terms, blocks):
    acc = None
    for sign, k, n in sorted(terms, reverse=True):
        v = blocks[k, n]
        if acc is None:
            acc = v if sign > 0 else -v
        else:
            acc = acc + v if sign > 0 else acc - v
    return acc


def _a_forms(x, y):
    x1, x2, x3 = x
    y1, y2, y3 = y
    s1 = x1 + y1
    s2 = x2 + y2
    f13 = s1 - y3
    f23 = s2 - x3
    return {1: x1, 2: s1, 3: s2, 4: y2, 5: x3, 6: y3, 7: x1 + y2, 8: x1 - x2, 9: y1 - y2,
            10: f13, 11: y1 - y3, 12: f13 - x3, 13: f23, 14: x2 - x3, 15: f23 - y3}


def _scheme_pass1(product, out, order):
    groups, swaps = order
    p = {}

    def issue(i):
        for r in groups[i]:
            p[r] = product(r)

    def emit(i, a, b):
        for o in ((b, a) if swaps[i] else (a, b)):
            out(*o)

    issue(0)
    g13 = p[10] + p[11]
    d1 = p[1] + g13
    t1 = d1 + p[12]
    t2 = g13 + p[12]
    issue(1)
    emit(0, (p[5] - t2 - p[14], 0, 2), (t1 + p[8], 0, 0))
    g23 = p[13] + p[14]
    v3 = p[11] + g23
    issue(2)
    d2 = g23 + p[4]
    emit(1, (v3 + p[6] - p[15], 1, 2), (p[9] + p[15] - d2, 1, 1))
    v1 = p[9] - d1
    u2 = d2 + p[8]
    issue(3)
    emit(2, (v1 + p[2] + p[7], 1, 0), (u2 + p[3] + p[7], 0, 1))


def _scheme_pass2(pair, single, out):
    def chain(a, b, c):
        def f(ld):
            e = _f32(ld(*b)) - _f32(ld(*c))
            return _bf16(_f32(ld(*a)) + e), _bf16(e)
        return f

    def sums(k):
        def f(ld):
            s = _f32(ld(0, k)) + _f32(ld(1, k))
            return _bf16(s), _bf16(s - (_f32(ld(0, 2)) + _f32(ld(1, 2))))
        return f

    def f78(ld):
        x1 = _f32(ld(0, 0))
        return _bf16(x1 + _f32(ld(1, 1))), _bf16(x1 - _f32(ld(0, 1)))

    p1, p5 = pair(1, 5, lambda ld: (ld(0, 0), ld(0, 2)))
    p10, p11 = pair(10, 11, chain((0, 0), (1, 0), (1, 2)))
    g13 = p10 + p11
    d1 = p1 + g13
    u3 = p5 - g13
    p2, p12 = pair(2, 12, sums(0))
    v1 = p2 - d1
    u1 = d1 + p12
    u3 = u3 - p12
    p4, p6 = pair(4, 6, lambda ld: (ld(1, 1), ld(1, 2)))
    v3 = p6 + p11
    p13, p14 = pair(13, 14, chain((1, 1), (0, 1), (0, 2)))
    g23 = p13 + p14
    d2 = p4 + g23
    v3 = v3 + g23
    out(u3 - p14, 0, 2)
    p3, p15 = pair(3, 15, sums(1))
    u2 = d2 + p3
    v2 = p15 - d2
    out(v3 - p15, 1, 2)
    p7, p8 = pair(7, 8, f78)
    out(u1 + p8, 0, 0)
    out(u2 + p7 + p8, 0, 1)
    v1 = v1 + p7
    p9 = single(9, lambda ld: _bf16(_f32(ld(1, 0)) - _f32(ld(1, 1))))
    out(v1 + p9, 1, 0)
    out(v2 + p9, 1, 1)


def _kernel(x_hbm, dw_hbm, w1_hbm, w2_hbm, g_hbm, b_hbm, o_hbm, h_hbm,
            hv, wf, w2v, xbuf, xp, af, xsem, osem, hsem, psem, wsem, esem, dw_v, g_v, b_v, ssem):
    N, C = x_hbm.shape
    F = w2v.shape[0]
    T = N // TM
    PS = 2 * PR
    NP = TM // PS
    J = T // U1

    def rows(ref, t):
        return ref.at[pl.ds(pl.multiple_of(t * TM, TM), TM)]

    def x_in(t):
        return pltpu.make_async_copy(rows(x_hbm, t), xbuf.at[t & 3], xsem.at[t & 3])

    def o_out(t):
        return pltpu.make_async_copy(xbuf.at[t & 3], rows(o_hbm, t), osem.at[t & 3])

    def p_in(j):
        src = x_hbm.at[pl.ds(pl.multiple_of(j * U1 * TM, TM), PS)]
        return pltpu.make_async_copy(src, xp.at[j & 1], psem.at[j & 1])

    def h_out(t, slot):
        return pltpu.make_async_copy(hv.at[slot], h_hbm.at[t], hsem.at[slot])

    def h_in(t, slot):
        return pltpu.make_async_copy(h_hbm.at[t], hv.at[slot], hsem.at[slot])

    def nxt(slot):
        return jnp.where(slot == S - 1, 0, slot + 1)

    def prv(slot):
        return jnp.where(slot == 0, S - 1, slot - 1)

    wf32, hv32, af32 = wf.bitcast(U32), hv.bitcast(U32), af.bitcast(U32)

    def w_tile(r, g):
        return _words(wf32[r - 1, g * (L // 2):(g + 1) * (L // 2), :])

    def store_b_forms(g, blocks):
        for r, terms in enumerate(_B_FORMS):
            wf[r, g * L:(g + 1) * L, :] = _bf16(_b_form(terms, blocks))

    w1_in = [pltpu.make_async_copy(w1_hbm.at[:, pl.ds(j * L, L)], hv.at[S - 1, j, pl.ds(0, C)], wsem.at[j % 4])
             for j in range(F // L)]
    w2_in = pltpu.make_async_copy(w2_hbm, w2v, wsem.at[4])
    dw_in, g_in, b_in = [pltpu.make_async_copy(src, dst, ssem.at[i])
                         for i, (src, dst) in enumerate(((dw_hbm, dw_v), (g_hbm, g_v), (b_hbm, b_v)))]
    p_in(0).start()
    dw_in.start()
    for g in range(4):
        for n in range(3):
            w1_in[4 * n + g].start()
    x_in(0).start()
    x_in(1).start()
    p_in(1).start()
    x_in(2).start()
    x_in(3).start()
    w2_in.start()
    g_in.start()
    b_in.start()
    af[...] = jnp.zeros(af.shape, BF16)
    dw_in.wait()
    dwv = _f32(dw_v[...])

    def piece(xv, ring):
        o = _f32(xv) * dwv
        d = o - jnp.sum(o, axis=-1, keepdims=True) * (1.0 / C)
        v = jnp.sum(d * d, axis=-1, keepdims=True)
        xn = d * jnp.exp2(jnp.log2(v + C * 1e-5) * -0.5 + math.log2(_AL * math.sqrt(C)))
        forms = _a_forms([xn[:PR, k * L:(k + 1) * L] for k in range(3)],
                         [xn[PR:, k * L:(k + 1) * L] for k in range(3)])
        for r in range(1, 16):
            af[ring, r - 1] = _bf16(forms[r])

    def unit(u, pieces, slots, sumsq):
        g = u % 4

        def product(r):
            a = jnp.concatenate([af32[q % 4, r - 1] for q in pieces], axis=0)
            return jnp.dot(_words(a), w_tile(r, g), preferred_element_type=F32)

        def out(y, m, n):
            j = 4 * n + g
            h = y + y * jnp.tanh(y * (y * y + _CC))
            hb = _bf16(h)
            for i, q in enumerate(pieces):
                hv[slots[q // NP], j, pl.ds(((q % NP) * 2 + m) * PR, PR), :] = hb[i * PR:(i + 1) * PR]
            sumsq[j] = sumsq[j] + jnp.sum((h * h).reshape(-1, 8, L), axis=0)

        _scheme_pass1(product, out, _ORDER[u % 4])

    p_in(0).wait()
    piece(xp[0], 0)
    p_in(2).start()
    for g in range(4):
        for n in range(3):
            w1_in[4 * n + g].wait()
        store_b_forms(g, {(k, n): _f32(hv[S - 1, 4 * n + g, k * L:(k + 1) * L, :])
                          for k in range(3) for n in range(3)})

    def step1(j, carry):
        s0, acc = carry
        t0 = j * U1
        slots = {-1: prv(s0), 0: s0, 1: nxt(s0)}
        sumsq = list(acc)
        s2 = nxt(slots[1])
        for u in range(U1 * NP):
            unit(u, [u, u - 1, u - 2, u - 3], slots, sumsq)
            q = u + 1
            if q < U1 * NP:
                piece(xbuf[(t0 + q // NP) & 3, pl.ds((q % NP) * PS, PS), :], q % 4)
            else:
                piece(xp[(j + 1) & 1], 0)

        for e in (-1, 0):
            @pl.when(jnp.logical_and(t0 + e >= 0, t0 + e < T - S))
            def _():
                h_out(t0 + e, slots[e]).start()

        @pl.when(j + 2 < J)
        def _():
            for e in range(U1):
                x_in(t0 + 2 * U1 + e).start()

        @pl.when(j + 3 < J)
        def _():
            p_in(j + 3).start()

        @pl.when(j + 1 < J)
        def _():
            for e in range(U1):
                x_in(t0 + U1 + e).wait()

        @pl.when(j + 2 < J)
        def _():
            p_in(j + 2).wait()

        @pl.when(jnp.logical_and(t0 + U1 >= S, j + 1 < J))
        def _():
            h_out(t0 + U1 - S, s2).wait()
            h_out(t0 + U1 + 1 - S, nxt(s2)).wait()

        return s2, tuple(sumsq)

    acc = tuple(jnp.zeros((8, L), F32) for _ in range(F // L))
    x_in(0).wait()
    x_in(1).wait()
    p_in(1).wait()
    sumsq = list(lax.fori_loop(0, J, step1, (jnp.int32(0), acc))[1])
    for u in range(3):
        unit(u, list(range(u - 3, 0)), {-1: (T - 1) % S}, sumsq)
    w2_in.wait()
    g_in.wait()
    b_in.wait()

    ss = jnp.sum(jnp.concatenate(sumsq, axis=1), axis=0, keepdims=True)
    gx = jnp.sqrt(ss * (_HS * _HS) + 1e-6)
    nx = gx / (jnp.mean(gx, axis=-1, keepdims=True) + 1e-6)
    scale = (1.0 + _f32(g_v[...]).reshape(1, F) * nx) * _HS
    for g in range(4):
        blocks = {}
        for k in range(3):
            j = 4 * k + g
            col = jnp.transpose(jnp.broadcast_to(scale[:, j * L:(j + 1) * L], (L, L)))
            for n in range(3):
                blocks[k, n] = _f32(w2v[j * L:(j + 1) * L, n * L:(n + 1) * L]) * col
        store_b_forms(g, blocks)
    bias = jnp.dot(_bf16(jnp.broadcast_to(_f32(b_v[...]).reshape(1, F), (16, F))), w2v[...],
                   preferred_element_type=F32)[0:1]

    def chunk(i, slot, xs, r0, cm):
        def loader(r, g):
            sl = slot + (i >> (8 + r))

            def ld(m, k):
                span = pl.ds(pl.multiple_of((r0 + m * cm) // 2, cm // 2), cm // 2)
                return _words(hv32[sl, 4 * k + g, span, :])
            return ld

        def dot(a, r, g):
            return jnp.dot(a, w_tile(r, g), preferred_element_type=F32)

        def pair(ra, rb, forms):
            ya = yb = None
            for g in (0, 2):
                o = [forms(loader(ra, gg)) for gg in (g, g + 1)]
                a = dot(o[0][0], ra, g) + dot(o[1][0], ra, g + 1)
                b = dot(o[0][1], rb, g) + dot(o[1][1], rb, g + 1)
                ya, yb = (a, b) if ya is None else (ya + a, yb + b)
            return ya, yb

        def single(r, form):
            d = [dot(form(loader(r, g)), r, g) for g in range(4)]
            return (d[0] + d[1]) + (d[2] + d[3])

        def out(y, m, n):
            span = pl.ds(pl.multiple_of(r0 + m * cm, cm), cm)
            cols = slice(n * L, (n + 1) * L)
            xbuf[xs, span, cols] = _bf16(_f32(xbuf[xs, span, cols]) + bias[:, cols] + y)

        _scheme_pass2(pair, single, out)

    PE = TM // NE

    def part(c):
        return pl.ds(pl.multiple_of(c * PE, PE), PE)

    def h_in_part(t, slot, c, sem):
        return pltpu.make_async_copy(h_hbm.at[t, :, part(c)], hv.at[slot, :, part(c)], sem)

    def first(c, _):
        chunk(c, (T - 1) % S, (T - 1) & 3, c * PE, PE // 2)
        h_in_part(T - S - 1, (T - 1) % S, c, hsem.at[(T - 1) % S]).start(priority=1)

    lax.fori_loop(0, NE, first, None)

    def tile2(i, carry, closes_pair):
        slot, m, mslot, err = carry
        t = T - 1 - i
        for c in range(TM // (2 * CM)):
            chunk(i, slot, t & 3, 2 * c * CM, CM)
        if closes_pair:
            o_out(t + 1).start()
            o_out(t).start()
        err = err + (T - S)
        fetch = jnp.logical_and(err >= T - LEAD, m >= 0)

        @pl.when(jnp.logical_and(fetch, m > 0))
        def _():
            h_in(m, mslot).start(priority=1)

        @pl.when(jnp.logical_and(fetch, m == 0))
        def _():
            for c in range(NE):
                h_in_part(0, 0, c, esem.at[c]).start(priority=1)

        if closes_pair:
            @pl.when(i >= 3)
            def _():
                x_in(t - 1).wait()
                x_in(t - 2).wait()
        else:
            o_out(t + 2).wait()
            o_out(t + 1).wait()

            @pl.when(t >= 3)
            def _():
                x_in(t - 2).start()
                x_in(t - 3).start()

        @pl.when(jnp.logical_and(i >= S - 1, t >= 2))
        def _():
            h_in(t - 1, prv(slot)).wait()

        return (prv(slot), jnp.where(fetch, m - 1, m), jnp.where(fetch, prv(mslot), mslot),
                jnp.where(fetch, err - (T - LEAD), err))

    def step2(j, carry):
        return tile2(2 * j + 2, tile2(2 * j + 1, carry, True), False)

    lax.fori_loop(0, (T - 2) // 2, step2,
                  tuple(jnp.int32(v) for v in ((T - 2) % S, T - S - 2, (T - 2) % S, T - LEAD - 1)))
    o_out(1).start()

    def last(c, _):
        h_in_part(0, 0, c, esem.at[c]).wait()
        chunk(c, 0, 0, c * PE, PE // 2)
        pltpu.make_async_copy(xbuf.at[0, part(c)], o_hbm.at[part(c)], osem.at[0]).start()

    lax.fori_loop(0, NE, last, None)
    o_out(1).wait()
    o_out(0).wait()


@jax.jit
def pallas_standalone__modern_conv_block_slak__vision_kernel(x, dw, w1, w2, grn_g, grn_b):
    B, H, W, C = x.shape
    N = H * W
    F = w1.shape[1]
    T = N // TM
    assert B == 1 and dw.shape == (1, 1, C) and C == 3 * L and F == 4 * C
    assert N % (U1 * TM) == 0 and S % U1 == 0 and S + LEAD < T <= 256
    hbm = pl.BlockSpec(memory_space=pl.ANY)
    out, _ = pl.pallas_call(
        _kernel,
        in_specs=[hbm] * 6,
        out_specs=[hbm, hbm],
        out_shape=[jax.ShapeDtypeStruct((N, C), x.dtype),
                   jax.ShapeDtypeStruct((T - S, F // L, TM, L), BF16)],
        scratch_shapes=[
            pltpu.VMEM((S, F // L, TM, L), BF16),
            pltpu.VMEM((15, 4 * L, L), BF16),
            pltpu.VMEM((F, C), BF16),
            pltpu.VMEM((4, TM, C), BF16),
            pltpu.VMEM((2, 2 * PR, C), BF16),
            pltpu.VMEM((4, 15, PR, L), BF16),
            pltpu.SemaphoreType.DMA((4,)),
            pltpu.SemaphoreType.DMA((4,)),
            pltpu.SemaphoreType.DMA((S,)),
            pltpu.SemaphoreType.DMA((2,)),
            pltpu.SemaphoreType.DMA((5,)),
            pltpu.SemaphoreType.DMA((NE,)),
            pltpu.VMEM((1, C), dw.dtype),
            pltpu.VMEM((F,), grn_g.dtype),
            pltpu.VMEM((F,), grn_b.dtype),
            pltpu.SemaphoreType.DMA((3,)),
        ],
        compiler_params=pltpu.CompilerParams(vmem_limit_bytes=128 * 1024 * 1024, disable_bounds_checks=True),
    )(x.reshape(N, C), dw.reshape(1, C), w1, w2, grn_g, grn_b)
    return out.reshape(x.shape)
```

```python
import math

import jax
import jax.numpy as jnp
from jax import lax
from jax.experimental import pallas as pl
from jax.experimental.pallas import tpu as pltpu

F32, BF16, U32 = jnp.float32, jnp.bfloat16, jnp.uint32
L = 128
TM = 1024
S = 40
U1 = 2
PR = 32
CM = 256
NE = 2
LEAD = 10

_C0 = math.sqrt(2.0 / math.pi)
_AL = (0.044715 * _C0) ** (1.0 / 3.0)
_CC = _C0 / _AL
_HS = 0.5 / _AL

_B_FORMS = (
    ((1, 0, 0), (1, 0, 2), (1, 1, 0)),
    ((1, 0, 0), (-1, 0, 1), (1, 2, 0)),
    ((-1, 1, 0), (1, 1, 1), (1, 2, 1)),
    ((-1, 0, 1), (-1, 1, 1), (-1, 1, 2)),
    ((1, 1, 2), (1, 2, 0), (1, 2, 2)),
    ((1, 0, 2), (1, 2, 1), (1, 2, 2)),
    ((1, 0, 1), (1, 1, 0)),
    ((-1, 1, 0),),
    ((1, 0, 1),),
    ((-1, 0, 2), (1, 2, 0)),
    ((1, 0, 2),),
    ((-1, 2, 0),),
    ((1, 1, 2), (-1, 2, 1)),
    ((-1, 1, 2),),
    ((-1, 2, 1),),
)

_ORDER = (
    (11, 12, 1, 10, 14, 5, 13, 8, 15, 6, 4, 9, 3, 7, 2),
    (10, 12, 1, 11, 14, 5, 15, 13, 8, 6, 4, 9, 3, 2, 7),
    (10, 12, 1, 11, 5, 14, 13, 8, 15, 6, 4, 9, 3, 7, 2),
    (10, 11, 1, 12, 13, 5, 14, 8, 15, 6, 4, 9, 3, 7, 2),
)


def _bf16(v):
    return v.astype(BF16)


def _f32(v):
    return v.astype(F32)


def _words(v):
    return pltpu.bitcast(v, BF16)


def _b_form(terms, blocks):
    acc = None
    for sign, k, n in sorted(terms, reverse=True):
        v = blocks[k, n]
        if acc is None:
            acc = v if sign > 0 else -v
        else:
            acc = acc + v if sign > 0 else acc - v
    return acc


def _a_forms(x, y):
    x1, x2, x3 = x
    y1, y2, y3 = y
    s1 = x1 + y1
    s2 = x2 + y2
    f13 = s1 - y3
    f23 = s2 - x3
    return {1: x1, 2: s1, 3: s2, 4: y2, 5: x3, 6: y3, 7: x1 + y2, 8: x1 - x2, 9: y1 - y2,
            10: f13, 11: y1 - y3, 12: f13 - x3, 13: f23, 14: x2 - x3, 15: f23 - y3}


def _scheme_pass1(product, out, order):
    p = {}
    steps = [
        ("g13", (10, 11), lambda: p[10] + p[11]),
        ("d1", (1, "g13"), lambda: p[1] + p["g13"]),
        ("t1", ("d1", 12), lambda: p["d1"] + p[12]),
        ("t2", ("g13", 12), lambda: p["g13"] + p[12]),
        ((0, 0), ("t1", 8), lambda: p["t1"] + p[8]),
        ((0, 2), (5, "t2", 14), lambda: p[5] - p["t2"] - p[14]),
        ("g23", (13, 14), lambda: p[13] + p[14]),
        ("v3", (11, "g23"), lambda: p[11] + p["g23"]),
        ("d2", (4, "g23"), lambda: p["g23"] + p[4]),
        ((1, 1), (9, 15, "d2"), lambda: p[9] + p[15] - p["d2"]),
        ((1, 2), ("v3", 6, 15), lambda: p["v3"] + p[6] - p[15]),
        ("v1", (9, "d1"), lambda: p[9] - p["d1"]),
        ("u2", (8, "d2"), lambda: p["d2"] + p[8]),
        ((0, 1), ("u2", 3, 7), lambda: p["u2"] + p[3] + p[7]),
        ((1, 0), ("v1", 2, 7), lambda: p["v1"] + p[2] + p[7]),
    ]
    for r in order:
        p[r] = product(r)
        for name, needs, value in steps:
            if name not in p and all(k in p for k in needs):
                p[name] = value()
                if isinstance(name, tuple):
                    out(p[name], *name)


def _scheme_pass2(pair, single, out):
    def chain(a, b, c):
        def f(ld):
            e = _f32(ld(*b)) - _f32(ld(*c))
            return _bf16(_f32(ld(*a)) + e), _bf16(e)
        return f

    def sums(k):
        def f(ld):
            s = _f32(ld(0, k)) + _f32(ld(1, k))
            return _bf16(s), _bf16(s - (_f32(ld(0, 2)) + _f32(ld(1, 2))))
        return f

    def f78(ld):
        x1 = _f32(ld(0, 0))
        return _bf16(x1 + _f32(ld(1, 1))), _bf16(x1 - _f32(ld(0, 1)))

    p1, p5 = pair(1, 5, lambda ld: (ld(0, 0), ld(0, 2)))
    p10, p11 = pair(10, 11, chain((0, 0), (1, 0), (1, 2)))
    g13 = p10 + p11
    d1 = p1 + g13
    u3 = p5 - g13
    p2, p12 = pair(2, 12, sums(0))
    v1 = p2 - d1
    u1 = d1 + p12
    u3 = u3 - p12
    p4, p6 = pair(4, 6, lambda ld: (ld(1, 1), ld(1, 2)))
    v3 = p6 + p11
    p13, p14 = pair(13, 14, chain((1, 1), (0, 1), (0, 2)))
    g23 = p13 + p14
    d2 = p4 + g23
    v3 = v3 + g23
    out(u3 - p14, 0, 2)
    p3, p15 = pair(3, 15, sums(1))
    u2 = d2 + p3
    v2 = p15 - d2
    out(v3 - p15, 1, 2)
    p7, p8 = pair(7, 8, f78)
    out(u1 + p8, 0, 0)
    out(u2 + p7 + p8, 0, 1)
    v1 = v1 + p7
    p9 = single(9, lambda ld: _bf16(_f32(ld(1, 0)) - _f32(ld(1, 1))))
    out(v1 + p9, 1, 0)
    out(v2 + p9, 1, 1)


def _kernel(x_hbm, dw_hbm, w1_hbm, w2_hbm, g_hbm, b_hbm, o_hbm, h_hbm,
            hv, wf, w2v, xbuf, xp, af, xsem, osem, hsem, psem, wsem, esem, dw_v, g_v, b_v, ssem):
    N, C = x_hbm.shape
    F = w2v.shape[0]
    T = N // TM
    PS = 2 * PR
    NP = TM // PS
    J = T // U1

    def rows(ref, t):
        return ref.at[pl.ds(pl.multiple_of(t * TM, TM), TM)]

    def x_in(t):
        return pltpu.make_async_copy(rows(x_hbm, t), xbuf.at[t & 3], xsem.at[t & 3])

    def o_out(t):
        return pltpu.make_async_copy(xbuf.at[t & 3], rows(o_hbm, t), osem.at[t & 3])

    def p_in(j):
        src = x_hbm.at[pl.ds(pl.multiple_of(j * U1 * TM, TM), PS)]
        return pltpu.make_async_copy(src, xp.at[j & 1], psem.at[j & 1])

    def h_out(t, slot):
        return pltpu.make_async_copy(hv.at[slot], h_hbm.at[t], hsem.at[slot])

    def h_in(t, slot):
        return pltpu.make_async_copy(h_hbm.at[t], hv.at[slot], hsem.at[slot])

    def nxt(slot):
        return jnp.where(slot == S - 1, 0, slot + 1)

    def prv(slot):
        return jnp.where(slot == 0, S - 1, slot - 1)

    wf32, hv32, af32 = wf.bitcast(U32), hv.bitcast(U32), af.bitcast(U32)

    def w_tile(r, g):
        return _words(wf32[r - 1, g * (L // 2):(g + 1) * (L // 2), :])

    def store_b_forms(g, blocks):
        for r, terms in enumerate(_B_FORMS):
            wf[r, g * L:(g + 1) * L, :] = _bf16(_b_form(terms, blocks))

    w1_in = [pltpu.make_async_copy(w1_hbm.at[:, pl.ds(j * L, L)], hv.at[S - 1, j, pl.ds(0, C)], wsem.at[j % 4])
             for j in range(F // L)]
    w2_in = pltpu.make_async_copy(w2_hbm, w2v, wsem.at[4])
    dw_in, g_in, b_in = [pltpu.make_async_copy(src, dst, ssem.at[i])
                         for i, (src, dst) in enumerate(((dw_hbm, dw_v), (g_hbm, g_v), (b_hbm, b_v)))]
    p_in(0).start()
    dw_in.start()
    for g in range(4):
        for n in range(3):
            w1_in[4 * n + g].start()
    x_in(0).start()
    x_in(1).start()
    p_in(1).start()
    x_in(2).start()
    x_in(3).start()
    w2_in.start()
    g_in.start()
    b_in.start()
    af[...] = jnp.zeros(af.shape, BF16)
    dw_in.wait()
    dwv = _f32(dw_v[...])

    def piece(xv, ring):
        o = _f32(xv) * dwv
        d = o - jnp.sum(o, axis=-1, keepdims=True) * (1.0 / C)
        v = jnp.sum(d * d, axis=-1, keepdims=True)
        xn = d * jnp.exp2(jnp.log2(v + C * 1e-5) * -0.5 + math.log2(_AL * math.sqrt(C)))
        forms = _a_forms([xn[:PR, k * L:(k + 1) * L] for k in range(3)],
                         [xn[PR:, k * L:(k + 1) * L] for k in range(3)])
        for r in range(1, 16):
            af[ring, r - 1] = _bf16(forms[r])

    def unit(u, pieces, slots, sumsq):
        g = u % 4

        def product(r):
            a = jnp.concatenate([af32[q % 4, r - 1] for q in pieces], axis=0)
            return jnp.dot(_words(a), w_tile(r, g), preferred_element_type=F32)

        def out(y, m, n):
            j = 4 * n + g
            h = y + y * jnp.tanh(y * (y * y + _CC))
            hb = _bf16(h)
            for i, q in enumerate(pieces):
                hv[slots[q // NP], j, pl.ds(((q % NP) * 2 + m) * PR, PR), :] = hb[i * PR:(i + 1) * PR]
            sumsq[j] = sumsq[j] + jnp.sum((h * h).reshape(-1, 8, L), axis=0)

        _scheme_pass1(product, out, _ORDER[u % 4])

    p_in(0).wait()
    piece(xp[0], 0)
    p_in(2).start()
    for g in range(4):
        for n in range(3):
            w1_in[4 * n + g].wait()
        store_b_forms(g, {(k, n): _f32(hv[S - 1, 4 * n + g, k * L:(k + 1) * L, :])
                          for k in range(3) for n in range(3)})

    def step1(j, carry):
        s0, acc = carry
        t0 = j * U1
        slots = {-1: prv(s0), 0: s0, 1: nxt(s0)}
        sumsq = list(acc)
        s2 = nxt(slots[1])
        for u in range(U1 * NP):
            unit(u, [u, u - 1, u - 2, u - 3], slots, sumsq)
            q = u + 1
            if q < U1 * NP:
                piece(xbuf[(t0 + q // NP) & 3, pl.ds((q % NP) * PS, PS), :], q % 4)
            else:
                piece(xp[(j + 1) & 1], 0)

        for e in (-1, 0):
            @pl.when(jnp.logical_and(t0 + e >= 0, t0 + e < T - S))
            def _():
                h_out(t0 + e, slots[e]).start()

        @pl.when(j + 2 < J)
        def _():
            for e in range(U1):
                x_in(t0 + 2 * U1 + e).start()

        @pl.when(j + 3 < J)
        def _():
            p_in(j + 3).start()

        @pl.when(j + 1 < J)
        def _():
            for e in range(U1):
                x_in(t0 + U1 + e).wait()

        @pl.when(j + 2 < J)
        def _():
            p_in(j + 2).wait()

        @pl.when(jnp.logical_and(t0 + U1 >= S, j + 1 < J))
        def _():
            h_out(t0 + U1 - S, s2).wait()
            h_out(t0 + U1 + 1 - S, nxt(s2)).wait()

        return s2, tuple(sumsq)

    acc = tuple(jnp.zeros((8, L), F32) for _ in range(F // L))
    x_in(0).wait()
    x_in(1).wait()
    p_in(1).wait()
    sumsq = list(lax.fori_loop(0, J, step1, (jnp.int32(0), acc))[1])
    for u in range(3):
        unit(u, list(range(u - 3, 0)), {-1: (T - 1) % S}, sumsq)
    w2_in.wait()
    g_in.wait()
    b_in.wait()

    ss = jnp.sum(jnp.concatenate(sumsq, axis=1), axis=0, keepdims=True)
    gx = jnp.sqrt(ss * (_HS * _HS) + 1e-6)
    nx = gx / (jnp.mean(gx, axis=-1, keepdims=True) + 1e-6)
    scale = (1.0 + _f32(g_v[...]).reshape(1, F) * nx) * _HS
    for g in range(4):
        blocks = {}
        for k in range(3):
            j = 4 * k + g
            col = jnp.transpose(jnp.broadcast_to(scale[:, j * L:(j + 1) * L], (L, L)))
            for n in range(3):
                blocks[k, n] = _f32(w2v[j * L:(j + 1) * L, n * L:(n + 1) * L]) * col
        store_b_forms(g, blocks)
    bias = jnp.dot(_bf16(jnp.broadcast_to(_f32(b_v[...]).reshape(1, F), (16, F))), w2v[...],
                   preferred_element_type=F32)[0:1]

    def chunk(i, slot, xs, r0, cm):
        def loader(r, g):
            sl = slot + (i >> (8 + r))

            def ld(m, k):
                span = pl.ds(pl.multiple_of((r0 + m * cm) // 2, cm // 2), cm // 2)
                return _words(hv32[sl, 4 * k + g, span, :])
            return ld

        def dot(a, r, g):
            return jnp.dot(a, w_tile(r, g), preferred_element_type=F32)

        def pair(ra, rb, forms):
            ya = yb = None
            for g in (0, 2):
                o = [forms(loader(ra, gg)) for gg in (g, g + 1)]
                a = dot(o[0][0], ra, g) + dot(o[1][0], ra, g + 1)
                b = dot(o[0][1], rb, g) + dot(o[1][1], rb, g + 1)
                ya, yb = (a, b) if ya is None else (ya + a, yb + b)
            return ya, yb

        def single(r, form):
            d = [dot(form(loader(r, g)), r, g) for g in range(4)]
            return (d[0] + d[1]) + (d[2] + d[3])

        def out(y, m, n):
            span = pl.ds(pl.multiple_of(r0 + m * cm, cm), cm)
            cols = slice(n * L, (n + 1) * L)
            xbuf[xs, span, cols] = _bf16(_f32(xbuf[xs, span, cols]) + bias[:, cols] + y)

        _scheme_pass2(pair, single, out)

    PE = TM // NE

    def part(c):
        return pl.ds(pl.multiple_of(c * PE, PE), PE)

    def h_in_part(t, slot, c, sem):
        return pltpu.make_async_copy(h_hbm.at[t, :, part(c)], hv.at[slot, :, part(c)], sem)

    def first(c, _):
        chunk(c, (T - 1) % S, (T - 1) & 3, c * PE, PE // 2)
        h_in_part(T - S - 1, (T - 1) % S, c, hsem.at[(T - 1) % S]).start(priority=1)

    lax.fori_loop(0, NE, first, None)

    def tile2(i, carry, closes_pair):
        slot, m, mslot, err = carry
        t = T - 1 - i
        for c in range(TM // (2 * CM)):
            chunk(i, slot, t & 3, 2 * c * CM, CM)
        if closes_pair:
            o_out(t + 1).start()
            o_out(t).start()
        err = err + (T - S)
        fetch = jnp.logical_and(err >= T - LEAD, m >= 0)

        @pl.when(jnp.logical_and(fetch, m > 0))
        def _():
            h_in(m, mslot).start(priority=1)

        @pl.when(jnp.logical_and(fetch, m == 0))
        def _():
            for c in range(NE):
                h_in_part(0, 0, c, esem.at[c]).start(priority=1)

        if closes_pair:
            @pl.when(i >= 3)
            def _():
                x_in(t - 1).wait()
                x_in(t - 2).wait()
        else:
            o_out(t + 2).wait()
            o_out(t + 1).wait()

            @pl.when(t >= 3)
            def _():
                x_in(t - 2).start()
                x_in(t - 3).start()

        @pl.when(jnp.logical_and(i >= S - 1, t >= 2))
        def _():
            h_in(t - 1, prv(slot)).wait()

        return (prv(slot), jnp.where(fetch, m - 1, m), jnp.where(fetch, prv(mslot), mslot),
                jnp.where(fetch, err - (T - LEAD), err))

    def step2(j, carry):
        return tile2(2 * j + 2, tile2(2 * j + 1, carry, True), False)

    lax.fori_loop(0, (T - 2) // 2, step2,
                  tuple(jnp.int32(v) for v in ((T - 2) % S, T - S - 2, (T - 2) % S, T - LEAD - 1)))
    o_out(1).start()

    def last(c, _):
        h_in_part(0, 0, c, esem.at[c]).wait()
        chunk(c, 0, 0, c * PE, PE // 2)
        pltpu.make_async_copy(xbuf.at[0, part(c)], o_hbm.at[part(c)], osem.at[0]).start()

    lax.fori_loop(0, NE, last, None)
    o_out(1).wait()
    o_out(0).wait()


@jax.jit
def pallas_standalone__modern_conv_block_slak__vision_kernel(x, dw, w1, w2, grn_g, grn_b):
    B, H, W, C = x.shape
    N = H * W
    F = w1.shape[1]
    T = N // TM
    assert B == 1 and dw.shape == (1, 1, C) and C == 3 * L and F == 4 * C
    assert N % (U1 * TM) == 0 and S % U1 == 0 and S + LEAD < T <= 256
    hbm = pl.BlockSpec(memory_space=pl.ANY)
    out, _ = pl.pallas_call(
        _kernel,
        in_specs=[hbm] * 6,
        out_specs=[hbm, hbm],
        out_shape=[jax.ShapeDtypeStruct((N, C), x.dtype),
                   jax.ShapeDtypeStruct((T - S, F // L, TM, L), BF16)],
        scratch_shapes=[
            pltpu.VMEM((S, F // L, TM, L), BF16),
            pltpu.VMEM((15, 4 * L, L), BF16),
            pltpu.VMEM((F, C), BF16),
            pltpu.VMEM((4, TM, C), BF16),
            pltpu.VMEM((2, 2 * PR, C), BF16),
            pltpu.VMEM((4, 15, PR, L), BF16),
            pltpu.SemaphoreType.DMA((4,)),
            pltpu.SemaphoreType.DMA((4,)),
            pltpu.SemaphoreType.DMA((S,)),
            pltpu.SemaphoreType.DMA((2,)),
            pltpu.SemaphoreType.DMA((5,)),
            pltpu.SemaphoreType.DMA((NE,)),
            pltpu.VMEM((1, C), dw.dtype),
            pltpu.VMEM((F,), grn_g.dtype),
            pltpu.VMEM((F,), grn_b.dtype),
            pltpu.SemaphoreType.DMA((3,)),
        ],
        compiler_params=pltpu.CompilerParams(vmem_limit_bytes=128 * 1024 * 1024, disable_bounds_checks=True),
    )(x.reshape(N, C), dw.reshape(1, C), w1, w2, grn_g, grn_b)
    return out.reshape(x.shape)
```

```python
import math

import jax
import jax.numpy as jnp
from jax import lax
from jax.experimental import pallas as pl
from jax.experimental.pallas import tpu as pltpu

F32, BF16, U32 = jnp.float32, jnp.bfloat16, jnp.uint32
L = 128
TM = 1024
S = 40
U1 = 4
NX = 6
PR = 32
CM = 128
NE = 4
LEAD = 10

_C0 = math.sqrt(2.0 / math.pi)
_AL = (0.044715 * _C0) ** (1.0 / 3.0)
_CC = _C0 / _AL
_HS = 0.5 / _AL

_B_FORMS = (
    ((1, 0, 0), (1, 0, 2), (1, 1, 0)),
    ((1, 0, 0), (-1, 0, 1), (1, 2, 0)),
    ((-1, 1, 0), (1, 1, 1), (1, 2, 1)),
    ((-1, 0, 1), (-1, 1, 1), (-1, 1, 2)),
    ((1, 1, 2), (1, 2, 0), (1, 2, 2)),
    ((1, 0, 2), (1, 2, 1), (1, 2, 2)),
    ((1, 0, 1), (1, 1, 0)),
    ((-1, 1, 0),),
    ((1, 0, 1),),
    ((-1, 0, 2), (1, 2, 0)),
    ((1, 0, 2),),
    ((-1, 2, 0),),
    ((1, 1, 2), (-1, 2, 1)),
    ((-1, 1, 2),),
    ((-1, 2, 1),),
)

_ORDER = (
    (11, 12, 1, 10, 14, 5, 13, 8, 15, 6, 4, 9, 3, 7, 2),
    (10, 12, 1, 11, 14, 5, 15, 13, 8, 6, 4, 9, 3, 2, 7),
    (10, 12, 1, 11, 5, 14, 13, 8, 15, 6, 4, 9, 3, 7, 2),
    (10, 11, 1, 12, 13, 5, 14, 8, 15, 6, 4, 9, 3, 7, 2),
)


def _bf16(v):
    return v.astype(BF16)


def _f32(v):
    return v.astype(F32)


def _words(v):
    return pltpu.bitcast(v, BF16)


def _b_form(terms, blocks):
    acc = None
    for sign, k, n in sorted(terms, reverse=True):
        v = blocks[k, n]
        if acc is None:
            acc = v if sign > 0 else -v
        else:
            acc = acc + v if sign > 0 else acc - v
    return acc


def _a_forms(x, y):
    x1, x2, x3 = x
    y1, y2, y3 = y
    s1 = x1 + y1
    s2 = x2 + y2
    f13 = s1 - y3
    f23 = s2 - x3
    return {1: x1, 2: s1, 3: s2, 4: y2, 5: x3, 6: y3, 7: x1 + y2, 8: x1 - x2, 9: y1 - y2,
            10: f13, 11: y1 - y3, 12: f13 - x3, 13: f23, 14: x2 - x3, 15: f23 - y3}


def _scheme_pass1(product, out, order):
    p = {}
    steps = [
        ("g13", (10, 11), lambda: p[10] + p[11]),
        ("d1", (1, "g13"), lambda: p[1] + p["g13"]),
        ("t1", ("d1", 12), lambda: p["d1"] + p[12]),
        ("t2", ("g13", 12), lambda: p["g13"] + p[12]),
        ((0, 0), ("t1", 8), lambda: p["t1"] + p[8]),
        ((0, 2), (5, "t2", 14), lambda: p[5] - p["t2"] - p[14]),
        ("g23", (13, 14), lambda: p[13] + p[14]),
        ("v3", (11, "g23"), lambda: p[11] + p["g23"]),
        ("d2", (4, "g23"), lambda: p["g23"] + p[4]),
        ((1, 1), (9, 15, "d2"), lambda: p[9] + p[15] - p["d2"]),
        ((1, 2), ("v3", 6, 15), lambda: p["v3"] + p[6] - p[15]),
        ("v1", (9, "d1"), lambda: p[9] - p["d1"]),
        ("u2", (8, "d2"), lambda: p["d2"] + p[8]),
        ((0, 1), ("u2", 3, 7), lambda: p["u2"] + p[3] + p[7]),
        ((1, 0), ("v1", 2, 7), lambda: p["v1"] + p[2] + p[7]),
    ]
    for r in order:
        p[r] = product(r)
        for name, needs, value in steps:
            if name not in p and all(k in p for k in needs):
                p[name] = value()
                if isinstance(name, tuple):
                    out(p[name], *name)


def _scheme_pass2(pair, single, out):
    def chain(a, b, c):
        def f(ld):
            e = _f32(ld(*b)) - _f32(ld(*c))
            return _bf16(_f32(ld(*a)) + e), _bf16(e)
        return f

    def sums(k):
        def f(ld):
            s = _f32(ld(0, k)) + _f32(ld(1, k))
            return _bf16(s), _bf16(s - (_f32(ld(0, 2)) + _f32(ld(1, 2))))
        return f

    def f78(ld):
        x1 = _f32(ld(0, 0))
        return _bf16(x1 + _f32(ld(1, 1))), _bf16(x1 - _f32(ld(0, 1)))

    p1, p5 = pair(1, 5, lambda ld: (ld(0, 0), ld(0, 2)))
    p10, p11 = pair(10, 11, chain((0, 0), (1, 0), (1, 2)))
    g13 = p10 + p11
    d1 = p1 + g13
    u3 = p5 - g13
    p2, p12 = pair(2, 12, sums(0))
    v1 = p2 - d1
    u1 = d1 + p12
    u3 = u3 - p12
    p4, p6 = pair(4, 6, lambda ld: (ld(1, 1), ld(1, 2)))
    v3 = p6 + p11
    p13, p14 = pair(13, 14, chain((1, 1), (0, 1), (0, 2)))
    g23 = p13 + p14
    d2 = p4 + g23
    v3 = v3 + g23
    out(u3 - p14, 0, 2)
    p3, p15 = pair(3, 15, sums(1))
    u2 = d2 + p3
    v2 = p15 - d2
    out(v3 - p15, 1, 2)
    p7, p8 = pair(7, 8, f78)
    out(u1 + p8, 0, 0)
    out(u2 + p7 + p8, 0, 1)
    v1 = v1 + p7
    p9 = single(9, lambda ld: _bf16(_f32(ld(1, 0)) - _f32(ld(1, 1))))
    out(v1 + p9, 1, 0)
    out(v2 + p9, 1, 1)


def _kernel(x_hbm, dw_hbm, w1_hbm, w2_hbm, g_hbm, b_hbm, o_hbm, h_hbm,
            hv, wf, xbuf, xp, af, xsem, osem, hsem, psem, wsem, esem, dw_v, g_v, b_v, ssem):
    N, C = x_hbm.shape
    F = w2_hbm.shape[0]
    T = N // TM
    PS = 2 * PR
    NP = TM // PS
    J = T // U1

    def rows(ref, t):
        return ref.at[pl.ds(pl.multiple_of(t * TM, TM), TM)]

    def x_in(t, xs):
        return pltpu.make_async_copy(rows(x_hbm, t), xbuf.at[xs], xsem.at[xs])

    def o_out(t, xs):
        return pltpu.make_async_copy(xbuf.at[xs], rows(o_hbm, t), osem.at[xs])

    def xadd(xs, d):
        v = xs + d % NX
        return jnp.where(v >= NX, v - NX, v)

    def p_in(j):
        src = x_hbm.at[pl.ds(pl.multiple_of(j * U1 * TM, TM), PS)]
        return pltpu.make_async_copy(src, xp.at[j & 1], psem.at[j & 1])

    def h_out(t, slot):
        return pltpu.make_async_copy(hv.at[slot], h_hbm.at[t], hsem.at[slot])

    def h_in(t, slot):
        return pltpu.make_async_copy(h_hbm.at[t], hv.at[slot], hsem.at[slot])

    def prv(slot):
        return jnp.where(slot == 0, S - 1, slot - 1)

    wf32, hv32, af32 = wf.bitcast(U32), hv.bitcast(U32), af.bitcast(U32)

    def w_tile(r, g):
        return _words(wf32[r - 1, g * (L // 2):(g + 1) * (L // 2), :])

    def store_b_forms(g, blocks):
        for r, terms in enumerate(_B_FORMS):
            wf[r, g * L:(g + 1) * L, :] = _bf16(_b_form(terms, blocks))

    w1_in = [pltpu.make_async_copy(w1_hbm.at[:, pl.ds(j * L, L)], hv.at[S - 1, j, pl.ds(0, C)], wsem.at[j % 4])
             for j in range(F // L)]
    FH = F // 2
    w2_in = [pltpu.make_async_copy(w2_hbm.at[pl.ds(i * FH, FH)], xbuf.at[(T + i) % NX, pl.ds(0, FH)],
                                   xsem.at[(T + i) % NX]) for i in range(2)]

    def w2_rows(r0, n, cols):
        return xbuf[(T + r0 // FH) % NX, pl.ds(r0 % FH, n), cols]

    dw_in, g_in, b_in = [pltpu.make_async_copy(src, dst, ssem.at[i])
                         for i, (src, dst) in enumerate(((dw_hbm, dw_v), (g_hbm, g_v), (b_hbm, b_v)))]
    p_in(0).start()
    dw_in.start()
    for g in range(4):
        for n in range(3):
            w1_in[4 * n + g].start()
    for t in range(U1):
        x_in(t, t).start()
    p_in(1).start()
    for t in range(U1, NX):
        x_in(t, t).start()
    g_in.start()
    b_in.start()
    af[...] = jnp.zeros(af.shape, BF16)
    dw_in.wait()
    dwv = _f32(dw_v[...])

    def piece(xv, ring):
        o = _f32(xv) * dwv
        d = o - jnp.sum(o, axis=-1, keepdims=True) * (1.0 / C)
        v = jnp.sum(d * d, axis=-1, keepdims=True)
        xn = d * jnp.exp2(jnp.log2(v + C * 1e-5) * -0.5 + math.log2(_AL * math.sqrt(C)))
        forms = _a_forms([xn[:PR, k * L:(k + 1) * L] for k in range(3)],
                         [xn[PR:, k * L:(k + 1) * L] for k in range(3)])
        for r in range(1, 16):
            af[ring, r - 1] = _bf16(forms[r])

    def unit(u, pieces, slots, sumsq):
        g = u % 4

        def product(r):
            a = jnp.concatenate([af32[q % 4, r - 1] for q in pieces], axis=0)
            return jnp.dot(_words(a), w_tile(r, g), preferred_element_type=F32)

        def out(y, m, n):
            j = 4 * n + g
            h = y + y * jnp.tanh(y * (y * y + _CC))
            hb = _bf16(h)
            for i, q in enumerate(pieces):
                hv[slots[q // NP], j, pl.ds(((q % NP) * 2 + m) * PR, PR), :] = hb[i * PR:(i + 1) * PR]
            sumsq[j] = sumsq[j] + jnp.sum((h * h).reshape(-1, 8, L), axis=0)

        _scheme_pass1(product, out, _ORDER[u % 4])

    p_in(0).wait()
    piece(xp[0], 0)
    p_in(2).start()
    for g in range(4):
        for n in range(3):
            w1_in[4 * n + g].wait()
        store_b_forms(g, {(k, n): _f32(hv[S - 1, 4 * n + g, k * L:(k + 1) * L, :])
                          for k in range(3) for n in range(3)})

    def step1(j, carry):
        s0, x0, acc = carry
        t0 = j * U1
        slots = {e: s0 + e for e in range(U1)}
        slots[-1] = prv(s0)
        xs = [xadd(x0, e) for e in range(NX)]
        sumsq = list(acc)
        for u in range(U1 * NP):
            unit(u, [u, u - 1, u - 2, u - 3], slots, sumsq)
            q = u + 1
            if q < U1 * NP:
                piece(xbuf[xs[q // NP], pl.ds((q % NP) * PS, PS), :], q % 4)
            else:
                piece(xp[(j + 1) & 1], 0)
            if q % NP == NP - 1:
                @pl.when(t0 + q // NP + NX < T)
                def _():
                    x_in(t0 + q // NP + NX, xs[q // NP]).start()

        for e in range(-1, U1 - 1):
            @pl.when(jnp.logical_and(t0 + e >= 0, t0 + e < T - S))
            def _():
                h_out(t0 + e, slots[e]).start()

        @pl.when(j + 3 < J)
        def _():
            p_in(j + 3).start()

        @pl.when(j == J - 2)
        def _():
            for cp in w2_in:
                cp.start()

        @pl.when(j + 1 < J)
        def _():
            for e in range(U1, 2 * U1):
                x_in(t0 + e, xs[e % NX]).wait()

        @pl.when(j + 2 < J)
        def _():
            p_in(j + 2).wait()

        s1 = jnp.where(s0 + U1 == S, 0, s0 + U1)

        @pl.when(jnp.logical_and(t0 + U1 >= S, j + 1 < J))
        def _():
            for e in range(U1):
                h_out(t0 + U1 + e - S, s1 + e).wait()

        return s1, xs[U1], tuple(sumsq)

    acc = tuple(jnp.zeros((8, L), F32) for _ in range(F // L))
    for t in range(U1):
        x_in(t, t).wait()
    p_in(1).wait()
    sumsq = list(lax.fori_loop(0, J, step1, (jnp.int32(0), jnp.int32(0), acc))[2])
    for u in range(3):
        unit(u, list(range(u - 3, 0)), {-1: (T - 1) % S}, sumsq)
    for cp in w2_in:
        cp.wait()
    g_in.wait()
    b_in.wait()

    ss = jnp.sum(jnp.concatenate(sumsq, axis=1), axis=0, keepdims=True)
    gx = jnp.sqrt(ss * (_HS * _HS) + 1e-6)
    nx = gx / (jnp.mean(gx, axis=-1, keepdims=True) + 1e-6)
    scale = (1.0 + _f32(g_v[...]).reshape(1, F) * nx) * _HS
    for g in range(4):
        blocks = {}
        for k in range(3):
            j = 4 * k + g
            col = jnp.transpose(jnp.broadcast_to(scale[:, j * L:(j + 1) * L], (L, L)))
            for n in range(3):
                blocks[k, n] = _f32(w2_rows(j * L, L, slice(n * L, (n + 1) * L))) * col
        store_b_forms(g, blocks)
    bb = _bf16(jnp.broadcast_to(_f32(b_v[...]).reshape(1, F), (16, F)))
    bias = sum(jnp.dot(bb[:, i * FH:(i + 1) * FH], w2_rows(i * FH, FH, slice(None)), preferred_element_type=F32)
               for i in range(2))[0:1]
    for t in (T - NX + 1, T - NX):
        x_in(t, t % NX).start()

    def chunk(i, slot, xs, r0, cm):
        def loader(r, g):
            sl = slot + (i >> (8 + r))

            def ld(m, k):
                span = pl.ds(pl.multiple_of((r0 + m * cm) // 2, cm // 2), cm // 2)
                return _words(hv32[sl, 4 * k + g, span, :])
            return ld

        def dot(a, r, g):
            return jnp.dot(a, w_tile(r, g), preferred_element_type=F32)

        def pair(ra, rb, forms):
            ya = yb = None
            for g in (0, 2):
                o = [forms(loader(ra, gg)) for gg in (g, g + 1)]
                a = dot(o[0][0], ra, g) + dot(o[1][0], ra, g + 1)
                b = dot(o[0][1], rb, g) + dot(o[1][1], rb, g + 1)
                ya, yb = (a, b) if ya is None else (ya + a, yb + b)
            return ya, yb

        def single(r, form):
            d = [dot(form(loader(r, g)), r, g) for g in range(4)]
            return (d[0] + d[1]) + (d[2] + d[3])

        def out(y, m, n):
            span = pl.ds(pl.multiple_of(r0 + m * cm, cm), cm)
            cols = slice(n * L, (n + 1) * L)
            xbuf[xs, span, cols] = _bf16(_f32(xbuf[xs, span, cols]) + bias[:, cols] + y)

        _scheme_pass2(pair, single, out)

    PE = TM // NE

    def part(c):
        return pl.ds(pl.multiple_of(c * PE, PE), PE)

    def h_in_part(t, slot, c, sem):
        return pltpu.make_async_copy(h_hbm.at[t, :, part(c)], hv.at[slot, :, part(c)], sem)

    def first(c, _):
        chunk(c, (T - 1) % S, (T - 1) % NX, c * PE, PE // 2)
        h_in_part(T - S - 1, (T - 1) % S, c, hsem.at[(T - 1) % S]).start(priority=1)

    lax.fori_loop(0, NE, first, None)

    def tile2(i, carry, closes_pair):
        slot, xs, m, mslot, err = carry
        t = T - 1 - i
        for c in range(TM // (2 * CM)):
            chunk(i, slot, xs, 2 * c * CM, CM)
        if closes_pair:
            o_out(t + 1, xadd(xs, 1)).start()
            o_out(t, xs).start()
        err = err + (T - S)
        fetch = jnp.logical_and(err >= T - LEAD, m >= 0)

        @pl.when(jnp.logical_and(fetch, m > 0))
        def _():
            h_in(m, mslot).start(priority=1)

        @pl.when(jnp.logical_and(fetch, m == 0))
        def _():
            for c in range(NE):
                h_in_part(0, 0, c, esem.at[c]).start(priority=1)

        if closes_pair:
            @pl.when(i >= 3)
            def _():
                x_in(t - 1, xadd(xs, -1)).wait()
                x_in(t - 2, xadd(xs, -2)).wait()
        else:
            o_out(t + 2, xadd(xs, 2)).wait()
            o_out(t + 1, xadd(xs, 1)).wait()

            @pl.when(t + 1 >= NX)
            def _():
                x_in(t + 2 - NX, xadd(xs, 2)).start()
                x_in(t + 1 - NX, xadd(xs, 1)).start()

        @pl.when(jnp.logical_and(i >= S - 1, t >= 2))
        def _():
            h_in(t - 1, prv(slot)).wait()

        return (prv(slot), xadd(xs, -1), jnp.where(fetch, m - 1, m), jnp.where(fetch, prv(mslot), mslot),
                jnp.where(fetch, err - (T - LEAD), err))

    def step2(j, carry):
        return tile2(2 * j + 2, tile2(2 * j + 1, carry, True), False)

    lax.fori_loop(0, (T - 2) // 2, step2,
                  tuple(jnp.int32(v) for v in ((T - 2) % S, (T - 2) % NX, T - S - 2, (T - 2) % S, T - LEAD - 1)))
    o_out(1, 1).start()

    def last(c, _):
        h_in_part(0, 0, c, esem.at[c]).wait()
        chunk(c, 0, 0, c * PE, PE // 2)
        pltpu.make_async_copy(xbuf.at[0, part(c)], o_hbm.at[part(c)], osem.at[0]).start()

    lax.fori_loop(0, NE, last, None)
    o_out(1, 1).wait()
    o_out(0, 0).wait()


@jax.jit
def pallas_standalone__modern_conv_block_slak__vision_kernel(x, dw, w1, w2, grn_g, grn_b):
    B, H, W, C = x.shape
    N = H * W
    F = w1.shape[1]
    T = N // TM
    assert B == 1 and dw.shape == (1, 1, C) and C == 3 * L and F == 4 * C
    assert N % (U1 * TM) == 0 and S % U1 == 0 and S + LEAD < T <= 256
    hbm = pl.BlockSpec(memory_space=pl.ANY)
    out, _ = pl.pallas_call(
        _kernel,
        in_specs=[hbm] * 6,
        out_specs=[hbm, hbm],
        out_shape=[jax.ShapeDtypeStruct((N, C), x.dtype),
                   jax.ShapeDtypeStruct((T - S, F // L, TM, L), BF16)],
        scratch_shapes=[
            pltpu.VMEM((S, F // L, TM, L), BF16),
            pltpu.VMEM((15, 4 * L, L), BF16),
            pltpu.VMEM((NX, TM, C), BF16),
            pltpu.VMEM((2, 2 * PR, C), BF16),
            pltpu.VMEM((4, 15, PR, L), BF16),
            pltpu.SemaphoreType.DMA((NX,)),
            pltpu.SemaphoreType.DMA((NX,)),
            pltpu.SemaphoreType.DMA((S,)),
            pltpu.SemaphoreType.DMA((2,)),
            pltpu.SemaphoreType.DMA((4,)),
            pltpu.SemaphoreType.DMA((NE,)),
            pltpu.VMEM((1, C), dw.dtype),
            pltpu.VMEM((F,), grn_g.dtype),
            pltpu.VMEM((F,), grn_b.dtype),
            pltpu.SemaphoreType.DMA((3,)),
        ],
        compiler_params=pltpu.CompilerParams(vmem_limit_bytes=128 * 1024 * 1024, disable_bounds_checks=True),
    )(x.reshape(N, C), dw.reshape(1, C), w1, w2, grn_g, grn_b)
    return out.reshape(x.shape)
```

```python
import math

import jax
import jax.numpy as jnp
from jax import lax
from jax.experimental import pallas as pl
from jax.experimental.pallas import tpu as pltpu

F32, BF16, U32 = jnp.float32, jnp.bfloat16, jnp.uint32
L = 128
TM = 1024
S = 40
U1 = 4
NX = 6
PR = 32
CM = 128
NE = 4
LEAD = 10

_C0 = math.sqrt(2.0 / math.pi)
_AL = (0.044715 * _C0) ** (1.0 / 3.0)
_CC = _C0 / _AL
_HS = 0.5 / _AL

_B_FORMS = (
    ((1, 0, 0), (1, 0, 2), (1, 1, 0)),
    ((1, 0, 0), (-1, 0, 1), (1, 2, 0)),
    ((-1, 1, 0), (1, 1, 1), (1, 2, 1)),
    ((-1, 0, 1), (-1, 1, 1), (-1, 1, 2)),
    ((1, 1, 2), (1, 2, 0), (1, 2, 2)),
    ((1, 0, 2), (1, 2, 1), (1, 2, 2)),
    ((1, 0, 1), (1, 1, 0)),
    ((-1, 1, 0),),
    ((1, 0, 1),),
    ((-1, 0, 2), (1, 2, 0)),
    ((1, 0, 2),),
    ((-1, 2, 0),),
    ((1, 1, 2), (-1, 2, 1)),
    ((-1, 1, 2),),
    ((-1, 2, 1),),
)

_ORDER = (
    (12, 10, 1, 11, 14, 5, 8, 13, 15, 6, 4, 9, 3, 7, 2),
    (12, 10, 1, 11, 14, 5, 15, 13, 8, 6, 4, 9, 3, 2, 7),
    (12, 11, 1, 10, 5, 14, 8, 13, 15, 6, 4, 9, 3, 7, 2),
    (11, 10, 1, 12, 13, 5, 14, 8, 15, 6, 4, 9, 3, 7, 2),
)


def _bf16(v):
    return v.astype(BF16)


def _f32(v):
    return v.astype(F32)


def _words(v):
    return pltpu.bitcast(v, BF16)


def _b_form(terms, blocks):
    acc = None
    for sign, k, n in sorted(terms, reverse=True):
        v = blocks[k, n]
        if acc is None:
            acc = v if sign > 0 else -v
        else:
            acc = acc + v if sign > 0 else acc - v
    return acc


def _a_forms(x, y):
    x1, x2, x3 = x
    y1, y2, y3 = y
    s1 = x1 + y1
    s2 = x2 + y2
    f13 = s1 - y3
    f23 = s2 - x3
    return {1: x1, 2: s1, 3: s2, 4: y2, 5: x3, 6: y3, 7: x1 + y2, 8: x1 - x2, 9: y1 - y2,
            10: f13, 11: y1 - y3, 12: f13 - x3, 13: f23, 14: x2 - x3, 15: f23 - y3}


def _scheme_pass1(product, out, order):
    p = {}
    steps = [
        ("g13", (10, 11), lambda: p[10] + p[11]),
        ("d1", (1, "g13"), lambda: p[1] + p["g13"]),
        ("t1", ("d1", 12), lambda: p["d1"] + p[12]),
        ("t2", ("g13", 12), lambda: p["g13"] + p[12]),
        ((0, 0), ("t1", 8), lambda: p["t1"] + p[8]),
        ((0, 2), (5, "t2", 14), lambda: p[5] - p["t2"] - p[14]),
        ("g23", (13, 14), lambda: p[13] + p[14]),
        ("v3", (11, "g23"), lambda: p[11] + p["g23"]),
        ("d2", (4, "g23"), lambda: p["g23"] + p[4]),
        ((1, 1), (9, 15, "d2"), lambda: p[9] + p[15] - p["d2"]),
        ((1, 2), ("v3", 6, 15), lambda: p["v3"] + p[6] - p[15]),
        ("v1", (9, "d1"), lambda: p[9] - p["d1"]),
        ("u2", (8, "d2"), lambda: p["d2"] + p[8]),
        ((0, 1), ("u2", 3, 7), lambda: p["u2"] + p[3] + p[7]),
        ((1, 0), ("v1", 2, 7), lambda: p["v1"] + p[2] + p[7]),
    ]
    for r in order:
        p[r] = product(r)
        for name, needs, value in steps:
            if name not in p and all(k in p for k in needs):
                p[name] = value()
                if isinstance(name, tuple):
                    out(p[name], *name)


def _scheme_pass2(pair, single, out):
    def chain(a, b, c):
        def f(ld):
            e = _f32(ld(*b)) - _f32(ld(*c))
            return _bf16(_f32(ld(*a)) + e), _bf16(e)
        return f

    def sums(k):
        def f(ld):
            s = _f32(ld(0, k)) + _f32(ld(1, k))
            return _bf16(s), _bf16(s - (_f32(ld(0, 2)) + _f32(ld(1, 2))))
        return f

    def f78(ld):
        x1 = _f32(ld(0, 0))
        return _bf16(x1 + _f32(ld(1, 1))), _bf16(x1 - _f32(ld(0, 1)))

    p1, p5 = pair(1, 5, lambda ld: (ld(0, 0), ld(0, 2)))
    p10, p11 = pair(10, 11, chain((0, 0), (1, 0), (1, 2)))
    g13 = p10 + p11
    d1 = p1 + g13
    u3 = p5 - g13
    p2, p12 = pair(2, 12, sums(0))
    v1 = p2 - d1
    u1 = d1 + p12
    u3 = u3 - p12
    p4, p6 = pair(4, 6, lambda ld: (ld(1, 1), ld(1, 2)))
    v3 = p6 + p11
    p13, p14 = pair(13, 14, chain((1, 1), (0, 1), (0, 2)))
    g23 = p13 + p14
    d2 = p4 + g23
    v3 = v3 + g23
    out(u3 - p14, 0, 2)
    p3, p15 = pair(3, 15, sums(1))
    u2 = d2 + p3
    v2 = p15 - d2
    out(v3 - p15, 1, 2)
    p7, p8 = pair(7, 8, f78)
    out(u1 + p8, 0, 0)
    out(u2 + p7 + p8, 0, 1)
    v1 = v1 + p7
    p9 = single(9, lambda ld: _bf16(_f32(ld(1, 0)) - _f32(ld(1, 1))))
    out(v1 + p9, 1, 0)
    out(v2 + p9, 1, 1)


def _kernel(x_hbm, dw_hbm, w1_hbm, w2_hbm, g_hbm, b_hbm, o_hbm, h_hbm,
            hv, wf, xbuf, xp, af, xsem, osem, hsem, psem, wsem, esem, dw_v, g_v, b_v, ssem):
    N, C = x_hbm.shape
    F = w2_hbm.shape[0]
    T = N // TM
    PS = 2 * PR
    NP = TM // PS
    J = T // U1

    def rows(ref, t):
        return ref.at[pl.ds(pl.multiple_of(t * TM, TM), TM)]

    def x_in(t, xs):
        return pltpu.make_async_copy(rows(x_hbm, t), xbuf.at[xs], xsem.at[xs])

    def o_out(t, xs):
        return pltpu.make_async_copy(xbuf.at[xs], rows(o_hbm, t), osem.at[xs])

    def xadd(xs, d):
        v = xs + d % NX
        return jnp.where(v >= NX, v - NX, v)

    def p_in(j):
        src = x_hbm.at[pl.ds(pl.multiple_of(j * U1 * TM, TM), PS)]
        return pltpu.make_async_copy(src, xp.at[j & 1], psem.at[j & 1])

    def h_out(t, slot):
        return pltpu.make_async_copy(hv.at[slot], h_hbm.at[t], hsem.at[slot])

    def h_in(t, slot):
        return pltpu.make_async_copy(h_hbm.at[t], hv.at[slot], hsem.at[slot])

    def prv(slot):
        return jnp.where(slot == 0, S - 1, slot - 1)

    wf32, hv32, af32 = wf.bitcast(U32), hv.bitcast(U32), af.bitcast(U32)

    def w_tile(r, g):
        return _words(wf32[r - 1, g * (L // 2):(g + 1) * (L // 2), :])

    def store_b_forms(g, blocks):
        for r, terms in enumerate(_B_FORMS):
            wf[r, g * L:(g + 1) * L, :] = _bf16(_b_form(terms, blocks))

    w1_in = [pltpu.make_async_copy(w1_hbm.at[:, pl.ds(j * L, L)], hv.at[S - 1, j, pl.ds(0, C)], wsem.at[j % 4])
             for j in range(F // L)]
    FH = F // 2
    w2_in = [pltpu.make_async_copy(w2_hbm.at[pl.ds(i * FH, FH)], xbuf.at[(T + i) % NX, pl.ds(0, FH)],
                                   xsem.at[(T + i) % NX]) for i in range(2)]

    def w2_rows(r0, n, cols):
        return xbuf[(T + r0 // FH) % NX, pl.ds(r0 % FH, n), cols]

    dw_in, g_in, b_in = [pltpu.make_async_copy(src, dst, ssem.at[i])
                         for i, (src, dst) in enumerate(((dw_hbm, dw_v), (g_hbm, g_v), (b_hbm, b_v)))]
    p_in(0).start()
    dw_in.start()
    for g in range(4):
        for n in range(3):
            w1_in[4 * n + g].start()
    for t in range(U1):
        x_in(t, t).start()
    p_in(1).start()
    for t in range(U1, NX):
        x_in(t, t).start()
    g_in.start()
    b_in.start()
    af[...] = jnp.zeros(af.shape, BF16)
    dw_in.wait()
    dwv = _f32(dw_v[...])

    def piece(xv, ring):
        o = _f32(xv) * dwv
        d = o - jnp.sum(o, axis=-1, keepdims=True) * (1.0 / C)
        v = jnp.sum(d * d, axis=-1, keepdims=True)
        xn = d * jnp.exp2(jnp.log2(v + C * 1e-5) * -0.5 + math.log2(_AL * math.sqrt(C)))
        forms = _a_forms([xn[:PR, k * L:(k + 1) * L] for k in range(3)],
                         [xn[PR:, k * L:(k + 1) * L] for k in range(3)])
        for r in range(1, 16):
            af[ring, r - 1] = _bf16(forms[r])

    def unit(u, pieces, slots, sumsq):
        g = u % 4

        def product(r):
            a = jnp.concatenate([af32[q % 4, r - 1] for q in pieces], axis=0)
            return jnp.dot(_words(a), w_tile(r, g), preferred_element_type=F32)

        def out(y, m, n):
            j = 4 * n + g
            h = y + y * jnp.tanh(y * (y * y + _CC))
            hb = _bf16(h)
            for i, q in enumerate(pieces):
                hv[slots[q // NP], j, pl.ds(((q % NP) * 2 + m) * PR, PR), :] = hb[i * PR:(i + 1) * PR]
            sumsq[j] = sumsq[j] + jnp.sum((h * h).reshape(-1, 8, L), axis=0)

        _scheme_pass1(product, out, _ORDER[u % 4])

    p_in(0).wait()
    piece(xp[0], 0)
    p_in(2).start()
    for g in range(4):
        for n in range(3):
            w1_in[4 * n + g].wait()
        store_b_forms(g, {(k, n): _f32(hv[S - 1, 4 * n + g, k * L:(k + 1) * L, :])
                          for k in range(3) for n in range(3)})

    def step1(j, carry):
        s0, x0, acc = carry
        t0 = j * U1
        slots = {e: s0 + e for e in range(U1)}
        slots[-1] = prv(s0)
        xs = [xadd(x0, e) for e in range(NX)]
        sumsq = list(acc)
        for u in range(U1 * NP):
            unit(u, [u, u - 1, u - 2, u - 3], slots, sumsq)
            q = u + 1
            if q < U1 * NP:
                piece(xbuf[xs[q // NP], pl.ds((q % NP) * PS, PS), :], q % 4)
            else:
                piece(xp[(j + 1) & 1], 0)
            if q % NP == NP - 1:
                @pl.when(t0 + q // NP + NX < T)
                def _():
                    x_in(t0 + q // NP + NX, xs[q // NP]).start()

        for e in range(-1, U1 - 1):
            @pl.when(jnp.logical_and(t0 + e >= 0, t0 + e < T - S))
            def _():
                h_out(t0 + e, slots[e]).start()

        @pl.when(j + 3 < J)
        def _():
            p_in(j + 3).start()

        @pl.when(j == J - 2)
        def _():
            for cp in w2_in:
                cp.start()

        @pl.when(j + 1 < J)
        def _():
            for e in range(U1, 2 * U1):
                x_in(t0 + e, xs[e % NX]).wait()

        @pl.when(j + 2 < J)
        def _():
            p_in(j + 2).wait()

        s1 = jnp.where(s0 + U1 == S, 0, s0 + U1)

        @pl.when(jnp.logical_and(t0 + U1 >= S, j + 1 < J))
        def _():
            for e in range(U1):
                h_out(t0 + U1 + e - S, s1 + e).wait()

        return s1, xs[U1], tuple(sumsq)

    acc = tuple(jnp.zeros((8, L), F32) for _ in range(F // L))
    for t in range(U1):
        x_in(t, t).wait()
    p_in(1).wait()
    sumsq = list(lax.fori_loop(0, J, step1, (jnp.int32(0), jnp.int32(0), acc))[2])
    for u in range(3):
        unit(u, list(range(u - 3, 0)), {-1: (T - 1) % S}, sumsq)
    for cp in w2_in:
        cp.wait()
    g_in.wait()
    b_in.wait()

    ss = jnp.sum(jnp.concatenate(sumsq, axis=1), axis=0, keepdims=True)
    gx = jnp.sqrt(ss * (_HS * _HS) + 1e-6)
    nx = gx / (jnp.mean(gx, axis=-1, keepdims=True) + 1e-6)
    scale = (1.0 + _f32(g_v[...]).reshape(1, F) * nx) * _HS
    for g in range(4):
        blocks = {}
        for k in range(3):
            j = 4 * k + g
            col = jnp.transpose(jnp.broadcast_to(scale[:, j * L:(j + 1) * L], (L, L)))
            for n in range(3):
                blocks[k, n] = _f32(w2_rows(j * L, L, slice(n * L, (n + 1) * L))) * col
        store_b_forms(g, blocks)
    bb = _bf16(jnp.broadcast_to(_f32(b_v[...]).reshape(1, F), (16, F)))
    bias = sum(jnp.dot(bb[:, i * FH:(i + 1) * FH], w2_rows(i * FH, FH, slice(None)), preferred_element_type=F32)
               for i in range(2))[0:1]
    for t in (T - NX + 1, T - NX):
        x_in(t, t % NX).start()

    def chunk(i, slot, xs, r0, cm):
        def loader(r, g):
            sl = slot + (i >> (8 + r))

            def ld(m, k):
                span = pl.ds(pl.multiple_of((r0 + m * cm) // 2, cm // 2), cm // 2)
                return _words(hv32[sl, 4 * k + g, span, :])
            return ld

        def dot(a, r, g):
            return jnp.dot(a, w_tile(r, g), preferred_element_type=F32)

        def pair(ra, rb, forms):
            ya = yb = None
            for g in (0, 2):
                o = [forms(loader(ra, gg)) for gg in (g, g + 1)]
                a = dot(o[0][0], ra, g) + dot(o[1][0], ra, g + 1)
                b = dot(o[0][1], rb, g) + dot(o[1][1], rb, g + 1)
                ya, yb = (a, b) if ya is None else (ya + a, yb + b)
            return ya, yb

        def single(r, form):
            d = [dot(form(loader(r, g)), r, g) for g in range(4)]
            return (d[0] + d[1]) + (d[2] + d[3])

        def out(y, m, n):
            span = pl.ds(pl.multiple_of(r0 + m * cm, cm), cm)
            cols = slice(n * L, (n + 1) * L)
            xbuf[xs, span, cols] = _bf16(_f32(xbuf[xs, span, cols]) + bias[:, cols] + y)

        _scheme_pass2(pair, single, out)

    PE = TM // NE

    def part(c):
        return pl.ds(pl.multiple_of(c * PE, PE), PE)

    def h_in_part(t, slot, c, sem):
        return pltpu.make_async_copy(h_hbm.at[t, :, part(c)], hv.at[slot, :, part(c)], sem)

    def first(c, _):
        chunk(c, (T - 1) % S, (T - 1) % NX, c * PE, PE // 2)
        h_in_part(T - S - 1, (T - 1) % S, c, hsem.at[(T - 1) % S]).start(priority=1)

    lax.fori_loop(0, NE, first, None)

    def tile2(i, carry, closes_pair):
        slot, xs, m, mslot, err = carry
        t = T - 1 - i
        for c in range(TM // (2 * CM)):
            chunk(i, slot, xs, 2 * c * CM, CM)
        if closes_pair:
            o_out(t + 1, xadd(xs, 1)).start()
            o_out(t, xs).start()
        err = err + (T - S)
        fetch = jnp.logical_and(err >= T - LEAD, m >= 0)

        @pl.when(jnp.logical_and(fetch, m > 0))
        def _():
            h_in(m, mslot).start(priority=1)

        @pl.when(jnp.logical_and(fetch, m == 0))
        def _():
            for c in range(NE):
                h_in_part(0, 0, c, esem.at[c]).start(priority=1)

        if closes_pair:
            @pl.when(i >= 3)
            def _():
                x_in(t - 1, xadd(xs, -1)).wait()
                x_in(t - 2, xadd(xs, -2)).wait()
        else:
            o_out(t + 2, xadd(xs, 2)).wait()
            o_out(t + 1, xadd(xs, 1)).wait()

            @pl.when(t + 1 >= NX)
            def _():
                x_in(t + 2 - NX, xadd(xs, 2)).start()
                x_in(t + 1 - NX, xadd(xs, 1)).start()

        @pl.when(jnp.logical_and(i >= S - 1, t >= 2))
        def _():
            h_in(t - 1, prv(slot)).wait()

        return (prv(slot), xadd(xs, -1), jnp.where(fetch, m - 1, m), jnp.where(fetch, prv(mslot), mslot),
                jnp.where(fetch, err - (T - LEAD), err))

    def step2(j, carry):
        return tile2(2 * j + 2, tile2(2 * j + 1, carry, True), False)

    lax.fori_loop(0, (T - 2) // 2, step2,
                  tuple(jnp.int32(v) for v in ((T - 2) % S, (T - 2) % NX, T - S - 2, (T - 2) % S, T - LEAD - 1)))
    o_out(1, 1).start()

    def last(c, _):
        h_in_part(0, 0, c, esem.at[c]).wait()
        chunk(c, 0, 0, c * PE, PE // 2)
        pltpu.make_async_copy(xbuf.at[0, part(c)], o_hbm.at[part(c)], osem.at[0]).start()

    lax.fori_loop(0, NE, last, None)
    o_out(1, 1).wait()
    o_out(0, 0).wait()


@jax.jit
def pallas_standalone__modern_conv_block_slak__vision_kernel(x, dw, w1, w2, grn_g, grn_b):
    B, H, W, C = x.shape
    N = H * W
    F = w1.shape[1]
    T = N // TM
    assert B == 1 and dw.shape == (1, 1, C) and C == 3 * L and F == 4 * C
    assert N % (U1 * TM) == 0 and S % U1 == 0 and S + LEAD < T <= 256
    hbm = pl.BlockSpec(memory_space=pl.ANY)
    out, _ = pl.pallas_call(
        _kernel,
        in_specs=[hbm] * 6,
        out_specs=[hbm, hbm],
        out_shape=[jax.ShapeDtypeStruct((N, C), x.dtype),
                   jax.ShapeDtypeStruct((T - S, F // L, TM, L), BF16)],
        scratch_shapes=[
            pltpu.VMEM((S, F // L, TM, L), BF16),
            pltpu.VMEM((15, 4 * L, L), BF16),
            pltpu.VMEM((NX, TM, C), BF16),
            pltpu.VMEM((2, 2 * PR, C), BF16),
            pltpu.VMEM((4, 15, PR, L), BF16),
            pltpu.SemaphoreType.DMA((NX,)),
            pltpu.SemaphoreType.DMA((NX,)),
            pltpu.SemaphoreType.DMA((S,)),
            pltpu.SemaphoreType.DMA((2,)),
            pltpu.SemaphoreType.DMA((4,)),
            pltpu.SemaphoreType.DMA((NE,)),
            pltpu.VMEM((1, C), dw.dtype),
            pltpu.VMEM((F,), grn_g.dtype),
            pltpu.VMEM((F,), grn_b.dtype),
            pltpu.SemaphoreType.DMA((3,)),
        ],
        compiler_params=pltpu.CompilerParams(vmem_limit_bytes=128 * 1024 * 1024, disable_bounds_checks=True),
    )(x.reshape(N, C), dw.reshape(1, C), w1, w2, grn_g, grn_b)
    return out.reshape(x.shape)
```
